```python
import os as _os
_os.environ.setdefault("JAX_PLATFORMS", "cpu")
import jax
import jax.numpy as jnp

def _softmax(x, axis=-1):
    return jax.nn.softmax(x, axis=axis)
def _gelu(x):
    return jax.nn.gelu(x, approximate=True)
def _silu(x):
    return jax.nn.silu(x)
def _sigmoid(x):
    return jax.nn.sigmoid(x)
def _layernorm(x, axis=-1, eps=1e-5):
    m = jnp.mean(x, axis=axis, keepdims=True)
    v = jnp.var(x, axis=axis, keepdims=True)
    return (x - m) / jnp.sqrt(v + eps)
def _scatter_add(tgt, idx, src, axis=0):
    return tgt.at[idx].add(src)
def _segment_sum(src, seg, n):
    return jax.ops.segment_sum(src, seg, n)
class _Rng:
    def __init__(self, key):
        self._k = key
    def _next(self):
        self._k, sub = jax.random.split(self._k)
        return sub
    def normal(self, shape):
        return jax.random.normal(self._next(), shape, dtype=jnp.bfloat16)
    def randint(self, lo, hi, shape):
        return jax.random.randint(self._next(), shape, lo, hi, dtype=jnp.int32)
    def uniform(self, shape, lo=0.0, hi=1.0):
        return jax.random.uniform(self._next(), shape, jnp.bfloat16, lo, hi)
    def permutation(self, n):
        return jax.random.permutation(self._next(), n)


kernel_name = 'standalone__layernorm_linear__sampling'

def setup_inputs():
    _rng = _Rng(jax.random.key(int.from_bytes(__import__("os").urandom(4), "little")))
    _w = (lambda a: (lambda t: t.astype(jnp.bfloat16) if jnp.issubdtype(t.dtype, jnp.floating) else t)(jnp.asarray(a)))
    B, S, D = 1024, 32, 576
    return {
        "x": _w((lambda *s: _rng.normal(s) * 0.05)(B, S, D)),
        "g": _w((lambda *s: _rng.normal(s) * 0.05)(D) + 1.0),
        "b": _w((lambda *s: _rng.normal(s) * 0.05)(D)),
        "w": _w((lambda *s: _rng.normal(s) * 0.05)(D, D)),
    }

def reference(x, g, b, w):
    return (_layernorm(x, axis=-1) * g + b) @ w
```

```python
import functools
import jax
import jax.numpy as jnp
import jax.experimental.pallas as pl
import jax.experimental.pallas.tpu as pltpu

EPS = 1e-5
F32 = jnp.float32
BF16 = jnp.bfloat16
U32 = jnp.uint32
H = 256
NH = 288
KR = 80
CG = 256
HH = 128

def dot(a, b):
    return jnp.dot(a, b, preferred_element_type=F32)


def _kernel(x_hbm, g_ref, b_ref, w_ref, o_hbm, x_buf, o_buf, a_sc, ar_sc, t_sc, xsem, osem, *, sched, pieces, oprio, gpc):
    S, D, B = x_hbm.shape
    cg, h = CG, HH
    CW = cg * gpc
    CPS = B // CW
    NC = S * CPS

    def chunk_ref(ref, c):
        if CPS == 1:
            return ref.at[c]
        if isinstance(c, int):
            return ref.at[c // CPS, :, pl.ds((c % CPS) * CW, CW)]
        return ref.at[c // CPS, :, pl.ds(pl.multiple_of((c % CPS) * CW, CW), CW)]

    def x_copy(c):
        src = c if isinstance(c, int) and c < NC else (NC - 1 if isinstance(c, int) else 0)
        return pltpu.make_async_copy(chunk_ref(x_hbm, src), x_buf.at[c], xsem.at[c])

    for c in range(NC + 1):
        x_copy(c).start()

    w = w_ref[...]
    row = jax.lax.broadcasted_iota(jnp.int32, (16, D), 0)
    b16 = jnp.where(row == 0, b_ref[...].astype(F32), 0.0).astype(BF16)
    d = dot(b16, w)[0:1, :]
    dh = d.astype(BF16).astype(F32)
    dl = (d - dh).astype(BF16).astype(F32)
    row64 = jax.lax.broadcasted_iota(jnp.int32, (64, D), 0)
    ext = jnp.where(row64 == 0, dh, jnp.where(row64 == 1, dl, 0.0))
    wt = jnp.concatenate([w.astype(F32), ext], axis=0).T
    gf = g_ref[...].astype(F32)
    a = wt[:, :2 * H] * gf[:, :2 * H]
    a11 = a[:NH, :H]; a12 = a[:NH, H:]; a21 = a[NH:, :H]; a22 = a[NH:, H:]
    for k, v in enumerate([a11 + a22, a21 + a22, a11, a22, a11 + a12, a21 - a11, a12 - a22]):
        a_sc[k] = pltpu.bitcast(v.astype(BF16), U32)
    gr = jnp.concatenate([gf[:, 2 * H:], jnp.ones((1, 64), F32)], axis=1)
    ar_sc[...] = pltpu.bitcast((wt[:, 2 * H:] * gr).astype(BF16), U32)

    A = lambda k: pltpu.bitcast(a_sc[k], BF16)
    AR = lambda i: pltpu.bitcast(ar_sc[i * NH // 2:(i + 1) * NH // 2, 0:KR], BF16)

    class Stats:
        def __init__(self, c, j):
            self.s = c
            self.cs = slice(j * cg, (j + 1) * cg)
            self.c = None
            self.r = 0
        def piece(self, nrows):
            s, cs = self.s, self.cs
            if self.c is None:
                self.c = x_buf[s, 0:8, cs].astype(F32)[0:1, :]
            for r in range(self.r, self.r + nrows, 8):
                y = x_buf[s, r:r + 8, cs].astype(F32) - self.c
                if r == 0:
                    self.a1 = y; self.a2 = y * y
                else:
                    self.a1 = self.a1 + y; self.a2 = self.a2 + y * y
            self.r += nrows
            z = self.a1 + self.a2
            return (z[:, :h] + z[:, h:])[0:1, :]
        def final(self):
            assert self.r == D
            s1 = jnp.sum(self.a1, axis=0, keepdims=True) * (1.0 / D)
            s2 = jnp.sum(self.a2, axis=0, keepdims=True) * (1.0 / D)
            m = self.c + s1
            v = jnp.maximum(s2 - s1 * s1, 0.0)
            rs = jax.lax.rsqrt(v + EPS)
            return rs, m * rs

    def mm(s, j, rs, mr, st):
        c0 = j * cg
        r1, r2 = rs[:, :h], rs[:, h:]
        q1, q2 = mr[:, :h], mr[:, h:]
        p1 = r1 > 0; p2 = r2 > 0
        pcs = list(pieces)
        def R(p, r):
            n = pcs.pop(0)
            return jnp.where(p, r, st.piece(n)) if n else r
        R1 = lambda: R(p1, r1)
        R2 = lambda: R(p2, r2)
        def ld(k):
            x = x_buf[s, k * H:(k + 1) * H, c0:c0 + cg].astype(F32)
            return x[:, :h], x[:, h:]
        x11, _ = ld(0); x21, x22 = ld(1)
        m1 = dot(A(0), ((x11 * R1() - q1) + (x22 * r2 - q2)).astype(BF16))
        m4 = dot(A(3), ((x21 - x11) * R1()).astype(BF16))
        t_sc[0] = m1 + m4
        t_sc[3] = m1
        t_sc[2] = m4
        _, x12 = ld(0); _, x22 = ld(1)
        m5 = dot(A(4), (x22 * R2() - q2).astype(BF16))
        m3 = dot(A(2), ((x12 - x22) * R2()).astype(BF16))
        t_sc[0] = t_sc[0] - m5
        t_sc[1] = m3 + m5
        t_sc[3] = t_sc[3] + m3
        x11, x12 = ld(0)
        n11 = x11 * R1() - q1
        m2 = dot(A(1), n11.astype(BF16))
        m6 = dot(A(5), (n11 + (x12 * R2() - q2)).astype(BF16))
        t_sc[2] = t_sc[2] + m2
        t_sc[3] = t_sc[3] + (m6 - m2)
        x21, x22 = ld(1)
        m7 = dot(A(6), (x21 * R1() + x22 * r2 - (q1 + q2)).astype(BF16))
        xr = x_buf[s, 2 * H:D, c0:c0 + cg].astype(F32)
        rsx = jnp.concatenate([R1(), r2], axis=1)
        br = jnp.concatenate([(xr * rsx - mr).astype(BF16), jnp.ones((KR - (D - 2 * H), cg), BF16)], axis=0)
        rr1 = dot(AR(0), br)
        o_buf[s, 0:NH, c0:c0 + cg] = (jnp.concatenate([t_sc[0] + m7, t_sc[1]], axis=1) + rr1).astype(o_buf.dtype)
        rr2 = dot(AR(1), br)
        o_buf[s, NH:D, c0:c0 + cg] = (jnp.concatenate([t_sc[2], t_sc[3]], axis=1) + rr2).astype(o_buf.dtype)

    x_copy(0).wait()
    carry = []
    for j in range(gpc):
        st = Stats(0, j); st.piece(D)
        carry.extend(st.final())
    carry = tuple(carry)

    def block(c_first, n, n_next, carry):
        carry = list(carry)
        for u in range(n):
            c = c_first + u
            new = []
            for j in range(gpc):
                st = Stats(c + 1, j)
                mm(c, j, carry[2 * j], carry[2 * j + 1], st)
                new.extend(st.final())
            carry = new
            pltpu.make_async_copy(o_buf.at[c], chunk_ref(o_hbm, c), osem).start(priority=oprio)
        for u in range(n_next):
            x_copy(c_first + n + 1 + u).wait()
        return tuple(carry)

    for u in range(sched[0][0]):
        x_copy(1 + u).wait()
    c0 = 0
    for si, (n, cnt) in enumerate(sched):
        n_after = sched[si + 1][0] if si + 1 < len(sched) else 0
        if cnt > 1:
            if n_after == n or True:
                def body(it, carry, c0=c0, n=n):
                    cf = c0 + it * n
                    carry = block(cf, n, 0, carry)
                    @pl.when(it + 1 < cnt)
                    def _():
                        for u in range(n):
                            x_copy(cf + n + 1 + u).wait()
                    return carry
                carry = jax.lax.fori_loop(0, cnt, body, carry)
                for u in range(n_after):
                    x_copy(c0 + n * cnt + 1 + u).wait()
        else:
            carry = block(c0, n, n_after, carry)
        c0 += n * cnt
    assert c0 == NC
    pltpu.make_async_copy(o_buf, o_buf, osem).wait()


@functools.partial(jax.jit, static_argnames=("sched", "pieces", "oprio", "gpc"))
def pallas_standalone__layernorm_linear__sampling_kernel(x, g, b, w, sched=((1, 1), (2, 1), (5, 1), (8, 7)), pieces=(0, 0, 96, 96, 96, 96, 96, 96), oprio=0, gpc=2):
    B, S, D = x.shape
    xt = jnp.transpose(x, (1, 2, 0))
    CW = CG * gpc
    NC = S * B // CW
    sched = tuple(tuple(s) for s in sched)
    out_t = pl.pallas_call(
        functools.partial(_kernel, sched=sched, pieces=tuple(pieces), oprio=oprio, gpc=gpc),
        in_specs=[
            pl.BlockSpec(memory_space=pl.ANY),
            pl.BlockSpec(memory_space=pltpu.VMEM),
            pl.BlockSpec(memory_space=pltpu.VMEM),
            pl.BlockSpec(memory_space=pltpu.VMEM),
        ],
        out_specs=pl.BlockSpec(memory_space=pl.ANY),
        out_shape=jax.ShapeDtypeStruct((S, D, B), x.dtype),
        scratch_shapes=[
            pltpu.VMEM((NC + 1, D, CW), BF16),
            pltpu.VMEM((NC, D, CW), BF16),
            pltpu.VMEM((7, NH // 2, H), U32),
            pltpu.VMEM((NH, 128), U32),
            pltpu.VMEM((4, NH, 128), F32),
            pltpu.SemaphoreType.DMA((NC + 1,)),
            pltpu.SemaphoreType.DMA(()),
        ],
        compiler_params=pltpu.CompilerParams(
            vmem_limit_bytes=110 * 1024 * 1024,
        ),
    )(xt, g.reshape(1, D), b.reshape(1, D), w)
    return jnp.transpose(out_t, (2, 0, 1))
```

```python
import functools
import jax
import jax.numpy as jnp
import jax.experimental.pallas as pl
import jax.experimental.pallas.tpu as pltpu

EPS = 1e-5
F32 = jnp.float32
BF16 = jnp.bfloat16
U32 = jnp.uint32
H = 256
NH = 288
KR = 80
CG = 256
HH = 128
LOOK = 2

ORDERS = {
    0: (("M1", "M4"), ("M5", "M3"), ("M2", "M6"), ("M7", "R1"), ("R2",)),
    1: (("R1", "R2"), ("M1", "M4"), ("M5", "M3"), ("M2", "M6"), ("M7",)),
    2: (("R1",), ("M1", "M4"), ("M2", "M6"), ("M3", "R2"), ("M5", "M7")),
    3: (("M1", "M4"), ("M2", "M6"), ("M3", "R2"), ("R1",), ("M5", "M7")),
}
CONTRIB = (
    {"M1": 1, "M4": 1, "M5": -1, "M7": 1, "R1": 1},
    {"M3": 1, "M5": 1, "R1": 1},
    {"M2": 1, "M4": 1, "R2": 1},
    {"M1": 1, "M2": -1, "M3": 1, "M6": 1, "R2": 1},
)


def dot(a, b):
    return jnp.dot(a, b, preferred_element_type=F32)


def _kernel(x_hbm, g_hbm, b_hbm, w_hbm, o_hbm, x_buf, o_buf, w_buf, g_buf, b_buf, a_sc, ar_sc, t_sc, xsem, osem,
            *, sched, pieces, fpieces, lpieces, wstart, closed0, last_order, dbg, f12):
    S, D, B = x_hbm.shape
    cg, h = CG, HH
    GPS = B // cg
    NG = S * GPS

    blocks = []
    g = 0
    for n, cnt in sched:
        for _ in range(cnt):
            blocks.append((g, n)); g += n
    assert g == NG

    def segs(lo, hi):
        out = []
        g = lo
        while g < hi:
            s, j = divmod(g, GPS)
            if j == 0 and hi - g >= GPS:
                ns = (hi - g) // GPS
                out.append(('slabs', s, ns)); g += ns * GPS
            else:
                n = min(hi - g, GPS - j)
                out.append(('cols', s, j * cg, n * cg)); g += n
        return out
    sets = [(0, 1)]
    have = 1
    for bi, (g0, n) in enumerate(blocks):
        need = min(g0 + n + LOOK, NG)
        if g0 % GPS == 0 and n % GPS == 0:
            need = min(g0 + n + GPS, NG)
        if bi == 0 and closed0:
            need = g0 + n
        need = max(need, have)
        sets.append((have, need)); have = need

    class Dummy:
        def start(self): pass
        def wait(self): pass
    def seg_copy(sg, k):
        if 'noread' in dbg:
            return Dummy()
        if sg[0] == 'slabs':
            _, s0, ns = sg
            return pltpu.make_async_copy(x_hbm.at[pl.ds(s0, ns)], x_buf.at[pl.ds(s0, ns)], xsem.at[k])
        _, s, c0, nc = sg
        return pltpu.make_async_copy(x_hbm.at[s, :, pl.ds(c0, nc)], x_buf.at[s, :, pl.ds(c0, nc)], xsem.at[k])

    w_cp = pltpu.make_async_copy(w_hbm, w_buf, xsem.at[len(sets)])
    g_cp = pltpu.make_async_copy(g_hbm, g_buf, xsem.at[len(sets) + 1])
    b_cp = pltpu.make_async_copy(b_hbm, b_buf, xsem.at[len(sets) + 2])
    w_cp.start(); g_cp.start(); b_cp.start()
    for k, (lo, hi) in enumerate(sets):
        for sg in segs(lo, hi):
            if sg[0] == 'slabs':
                for q in range(sg[2]):
                    seg_copy(('slabs', sg[1] + q, 1), k).start()
            else:
                seg_copy(sg, k).start()

    def wait_set(k):
        for sg in segs(*sets[k]):
            seg_copy(sg, k).wait()

    w_cp.wait(); g_cp.wait(); b_cp.wait()

    w = w_buf[...]
    row = jax.lax.broadcasted_iota(jnp.int32, (16, D), 0)
    b16 = jnp.where(row == 0, b_buf[...].astype(F32).reshape(1, D), 0.0).astype(BF16)
    d = dot(b16, w)[0:1, :]
    dh = d.astype(BF16).astype(F32)
    dl = (d - dh).astype(BF16).astype(F32)
    row64 = jax.lax.broadcasted_iota(jnp.int32, (64, D), 0)
    ext = jnp.where(row64 == 0, dh, jnp.where(row64 == 1, dl, 0.0))
    wt = jnp.concatenate([w.astype(F32), ext], axis=0).T
    gf = g_buf[...].astype(F32).reshape(1, D)
    a = wt[:, :2 * H] * gf[:, :2 * H]
    a11 = a[:NH, :H]; a12 = a[:NH, H:]; a21 = a[NH:, :H]; a22 = a[NH:, H:]
    for k, v in enumerate([a11 + a22, a21 + a22, a11, a22, a11 + a12, a21 - a11, a12 - a22]):
        a_sc[k] = pltpu.bitcast(v.astype(BF16), U32)
    gr = jnp.concatenate([gf[:, 2 * H:], jnp.ones((1, 64), F32)], axis=1)
    ar_sc[...] = pltpu.bitcast((wt[:, 2 * H:] * gr).astype(BF16), U32)

    A = lambda k: pltpu.bitcast(a_sc[k], BF16)
    AR = lambda i: pltpu.bitcast(ar_sc[i * NH // 2:(i + 1) * NH // 2, 0:KR], BF16)

    class Stats:
        def __init__(self, s, j):
            self.s = s
            self.cs = slice(j * cg, (j + 1) * cg)
            self.c = None
            self.r = 0
        def piece(self, nrows):
            s, cs = self.s, self.cs
            if self.c is None:
                self.c = x_buf[s, 0:8, cs].astype(F32)[0:1, :]
            for r in range(self.r, self.r + nrows, 8):
                y = x_buf[s, r:r + 8, cs].astype(F32) - self.c
                if r == 0:
                    self.a1 = y; self.a2 = y * y
                else:
                    self.a1 = self.a1 + y; self.a2 = self.a2 + y * y
            self.r += nrows
            z = self.a1 + self.a2
            return (z[:, :h] + z[:, h:])[0:1, :]
        def final(self):
            assert self.r == D, self.r
            s1 = jnp.sum(self.a1, axis=0, keepdims=True) * (1.0 / D)
            s2 = jnp.sum(self.a2, axis=0, keepdims=True) * (1.0 / D)
            m = self.c + s1
            v = jnp.maximum(s2 - s1 * s1, 0.0)
            rs = jax.lax.rsqrt(v + EPS)
            return rs, m * rs

    def mm(s, j, rs, mr, sts, order, pcs_list, after_half=None):
        c0 = j * cg
        r1, r2 = rs[:, :h], rs[:, h:]
        q1, q2 = mr[:, :h], mr[:, h:]
        p1 = r1 > 0; p2 = r2 > 0
        slot = [0]
        def R(p, r):
            k = slot[0]; slot[0] += 1
            z = None
            for st, pcs in zip(sts, pcs_list):
                if pcs[k]:
                    zz = st.piece(pcs[k])
                    z = zz if z is None else z + zz
            return r if z is None else jnp.where(p, r, z)
        R1 = lambda: R(p1, r1)
        R2 = lambda: R(p2, r2)
        def ld(k):
            x = x_buf[s, k * H:(k + 1) * H, c0:c0 + cg].astype(F32)
            return x[:, :h], x[:, h:]
        cache = {}
        def product(name, rnd):
            if name == "M1":
                x11, _ = ld(0); _, x22 = ld(1)
                return dot(A(0), ((x11 * R1() - q1) + (x22 * r2 - q2)).astype(BF16))
            if name == "M4":
                x11, _ = ld(0); x21, _ = ld(1)
                return dot(A(3), ((x21 - x11) * R1()).astype(BF16))
            if name == "M5":
                _, x22 = ld(1)
                return dot(A(4), (x22 * R2() - q2).astype(BF16))
            if name == "M3":
                _, x12 = ld(0); _, x22 = ld(1)
                return dot(A(2), ((x12 - x22) * R2()).astype(BF16))
            if name == "M2":
                x11, _ = ld(0)
                cache["n11"] = x11 * R1() - q1
                return dot(A(1), cache["n11"].astype(BF16))
            if name == "M6":
                x11, x12 = ld(0)
                n11 = cache["n11"] if "M2" in rnd else x11 * r1 - q1
                return dot(A(5), (n11 + (x12 * R2() - q2)).astype(BF16))
            if name == "M7":
                x21, x22 = ld(1)
                return dot(A(6), (x21 * R1() + x22 * r2 - (q1 + q2)).astype(BF16))
            if "br" not in cache:
                xr = x_buf[s, 2 * H:D, c0:c0 + cg].astype(F32)
                rsx = jnp.concatenate([R1(), r2], axis=1)
                cache["br"] = jnp.concatenate([(xr * rsx - mr).astype(BF16), jnp.ones((KR - (D - 2 * H), cg), BF16)], axis=0)
            return dot(AR(0 if name == "R1" else 1), cache["br"])
        started = [False] * 4
        remaining = [set(c) for c in CONTRIB]
        stored = [False, False]
        for rnd in ORDERS[order]:
            res = {nm: product(nm, rnd) for nm in rnd}
            vals = {}
            for c in range(4):
                pos = None; neg = None
                for nm in rnd:
                    if nm not in CONTRIB[c]:
                        continue
                    v = res[nm]
                    if nm[0] == "R":
                        v = v[:, (c % 2) * h:(c % 2 + 1) * h]
                    if CONTRIB[c][nm] > 0:
                        pos = v if pos is None else pos + v
                    else:
                        neg = v
                    remaining[c].discard(nm)
                if pos is None and neg is None:
                    continue
                if started[c]:
                    if pos is not None and neg is not None:
                        acc = t_sc[c] + (pos - neg)
                    elif pos is not None:
                        acc = t_sc[c] + pos
                    else:
                        acc = t_sc[c] - neg
                else:
                    acc = pos if neg is None else (pos - neg if pos is not None else -neg)
                started[c] = True
                vals[c] = acc
            for hf in range(2):
                ca, cb = 2 * hf, 2 * hf + 1
                if not stored[hf] and not remaining[ca] and not remaining[cb]:
                    va = vals.pop(ca) if ca in vals else t_sc[ca]
                    vb = vals.pop(cb) if cb in vals else t_sc[cb]
                    o_buf[s, hf * NH:(hf + 1) * NH, c0:c0 + cg] = jnp.concatenate([va, vb], axis=1).astype(o_buf.dtype)
                    stored[hf] = True
                    if after_half: after_half(hf)
            for c, v in vals.items():
                t_sc[c] = v
        assert slot[0] == 8 and all(stored)

    def o_start(s, rows, cols):
        if 'nowrite' in dbg:
            return
        pltpu.make_async_copy(o_buf.at[s, rows, cols], o_hbm.at[s, rows, cols], osem).start()

    def block(s_base, j_base, n, carry, write, first=False, closed=False):
        carry = list(carry)
        for u in range(n):
            ds_, j = divmod(j_base + u, GPS)
            s = s_base + ds_
            def tgt(off):
                if closed and u + off >= n:
                    return None
                ds2, j2 = divmod(j_base + u + off, GPS)
                s2 = s_base + ds2
                if isinstance(s2, int):
                    return None if s2 >= S else Stats(s2, j2)
                return Stats(jnp.minimum(s2, S - 1) if ds2 * GPS + j2 >= n else s2, j2)
            order = 1 if u == 0 else 0
            pcs = fpieces if u == 0 else pieces
            if first and u == 0:
                sts = [tgt(1), tgt(2)]
                pl_ = [f12[0], f12[1]]
                if sts[1] is None:
                    pl_ = [f12[2], None]
            else:
                sts = [tgt(LOOK)]
                pl_ = [pcs]
            last_slab = (u >= n - GPS) and n >= GPS
            ah = None
            if write == 'fine' and last_slab and u == n - 1:
                ah = lambda hf, s=s, j=j: o_start(s, pl.ds(hf * NH, NH), pl.ds(j * cg, cg))
                order = last_order
                pl_ = [lpieces]
            act = [(st, p) for st, p in zip(sts, pl_) if st is not None]
            mm(s, j, carry[0], carry[1], [a_[0] for a_ in act], order, [a_[1] for a_ in act], ah)
            fin = [st.final() if st is not None else None for st in sts]
            if first and u == 0:
                carry = list(fin[0]) + (list(fin[1]) if fin[1] is not None else list(carry[:2]))
            else:
                carry = carry[2:] + (list(fin[0]) if fin[0] is not None else carry[:2])
            if write == 'fine':
                if last_slab:
                    if u < n - 1:
                        o_start(s, pl.ds(0, D), pl.ds(j * cg, cg))
                elif j == GPS - 1:
                    o_start(s, pl.ds(0, D), pl.ds(0, B))
        if write == 'end' and 'nowrite' not in dbg:
            assert j_base == 0 and n % GPS == 0
            for q in range(n // GPS):
                pltpu.make_async_copy(o_buf.at[s_base + q], o_hbm.at[s_base + q], osem).start()
        return tuple(carry)

    wait_set(0)
    st = Stats(0, 0); st.piece(D)
    carry = st.final()

    bi = 0
    g0 = 0
    for si, (n, cnt) in enumerate(sched):
        write = 'none' if g0 < wstart else ('fine' if si == len(sched) - 1 else 'end')
        if g0 == wstart and wstart > 0 and 'nowrite' not in dbg:
            assert wstart % GPS == 0
            for q in range(wstart // GPS):
                pltpu.make_async_copy(o_buf.at[q], o_hbm.at[q], osem).start()
        wait_set(bi + 1)
        if cnt == 1:
            first = bi == 0
            if bi == 1 and closed0:
                st = Stats(g0 // GPS, g0 % GPS); st.piece(D)
                carry = st.final()
                first = True
            carry = block(g0 // GPS, g0 % GPS, n, carry, write, first=first, closed=(bi == 0 and closed0))
        else:
            assert g0 % GPS == 0 and n % GPS == 0
            ns = n // GPS
            def body(it, carry, g0=g0, n=n, cnt=cnt, bi=bi, ns=ns, write=write):
                sb = g0 // GPS + it * ns
                carry = block(sb, 0, n, carry, write)
                sizes = [(sets[bi + 2 + q][1] - sets[bi + 2 + q][0]) // GPS for q in range(cnt - 1)]
                for sz in sorted(set(sizes)):
                    qs = [q for q, z in enumerate(sizes) if z == sz]
                    assert qs == list(range(qs[0], qs[-1] + 1))
                    if sz == 0 or 'noread' in dbg:
                        continue
                    @pl.when(jnp.logical_and(it >= qs[0], it <= qs[-1]))
                    def _(sz=sz):
                        pltpu.make_async_copy(x_hbm.at[pl.ds(0, sz)], x_buf.at[pl.ds(sb + ns + 1, sz)], xsem.at[bi + 2 + it]).wait()
                return carry
            carry = jax.lax.fori_loop(0, cnt, body, carry)
        bi += cnt
        g0 += n * cnt
    if 'nowrite' not in dbg:
        pltpu.make_async_copy(o_buf, o_hbm, osem).wait()


@functools.partial(jax.jit, static_argnames=("sched", "pieces", "fpieces", "lpieces", "wstart", "nobc", "closed0", "last_order", "dbg", "f12"))
def pallas_standalone__layernorm_linear__sampling_kernel(x, g, b, w, sched=((2, 1), (2, 1), (4, 1), (8, 1), (16, 7)), pieces=(0, 48, 72, 72, 96, 96, 96, 96),
             fpieces=(0, 0, 96, 96, 96, 96, 96, 96), lpieces=(0, 0, 96, 96, 96, 96, 96, 96), wstart=16, nobc=True, closed0=True,
             last_order=2, dbg="", f12=((0, 0, 192, 192, 192, 0, 0, 0), (0, 0, 0, 0, 0, 192, 192, 192), (0, 0, 120, 120, 120, 120, 96, 0))):
    B, S, D = x.shape
    xt = jnp.transpose(x, (1, 2, 0))
    sched = tuple(tuple(s) for s in sched)
    nblk = sum(c for _, c in sched)
    out_t = pl.pallas_call(
        functools.partial(_kernel, sched=sched, pieces=tuple(pieces), fpieces=tuple(fpieces), lpieces=tuple(lpieces),
                          wstart=wstart, closed0=closed0, last_order=last_order, dbg=dbg, f12=f12),
        in_specs=[pl.BlockSpec(memory_space=pl.ANY)] * 4,
        out_specs=pl.BlockSpec(memory_space=pl.ANY),
        out_shape=jax.ShapeDtypeStruct((S, D, B), x.dtype),
        scratch_shapes=[
            pltpu.VMEM((S, D, B), BF16),
            pltpu.VMEM((S, D, B), BF16),
            pltpu.VMEM((D, D), BF16),
            pltpu.VMEM((D,), BF16),
            pltpu.VMEM((D,), BF16),
            pltpu.VMEM((7, NH // 2, H), U32),
            pltpu.VMEM((NH, 128), U32),
            pltpu.VMEM((4, NH, 128), F32),
            pltpu.SemaphoreType.DMA((nblk + 4,)),
            pltpu.SemaphoreType.DMA(()),
        ],
        compiler_params=pltpu.CompilerParams(
            vmem_limit_bytes=110 * 1024 * 1024,
            disable_bounds_checks=nobc,
        ),
    )(xt, g, b, w)
    return jnp.transpose(out_t, (2, 0, 1))
```

```python
import jax
import jax.numpy as jnp
import jax.experimental.pallas as pl
import jax.experimental.pallas.tpu as pltpu

EPS = 1e-5
F32 = jnp.float32
BF16 = jnp.bfloat16
U32 = jnp.uint32

T = 128
H = 256
NH = 288
NQ = 144
KR = 80
SGW = 512

B_TERMS = {1: ((1, 0, 0), (1, 1, 1)), 2: ((1, 0, 0),), 3: ((1, 0, 1), (-1, 1, 1)), 4: ((1, 1, 0), (-1, 0, 0)),
           5: ((1, 1, 1),), 6: ((1, 0, 0), (1, 0, 1)), 7: ((1, 1, 0), (1, 1, 1))}
A_TERMS = {1: ((1, 0, 0), (1, 1, 1)), 2: ((1, 1, 0), (1, 1, 1)), 3: ((1, 0, 0),), 4: ((1, 1, 1),),
           5: ((1, 0, 0), (1, 0, 1)), 6: ((1, 1, 0), (-1, 0, 0)), 7: ((1, 0, 1), (-1, 1, 1))}
C_TERMS = {(0, 0): {1: 1, 4: 1, 5: -1, 7: 1}, (0, 1): {3: 1, 5: 1},
           (1, 0): {2: 1, 4: 1}, (1, 1): {1: 1, 2: -1, 3: 1, 6: 1}}

LVL2 = (2, 5, 3, 4)
LVL1 = (1, 6, 7)

RAMP = (1, 1, 2, 4)
LOOP_N, LOOP_CNT = 8, 7
W_ITER, W_SLAB = 2, 2


def _dot(a, b):
    return jnp.dot(a, b, preferred_element_type=F32)


def _lin(terms):
    terms = sorted(terms, key=lambda t: -t[0])
    assert terms[0][0] > 0
    acc = terms[0][1]
    for sg, v in terms[1:]:
        acc = acc + v if sg > 0 else acc - v
    return acc


def _make_plan(d):
    M = lambda i, g: ("M", i, g)
    U = lambda i, u: ("U", i, u)
    R = lambda nh, g: ("R", nh, g)
    inner = []
    for i in LVL2:
        inner += [[U(i, 1), U(i, 4), U(i, 5), U(i, 3)], [U(i, 2), U(i, 6), U(i, 7)]]
    m16 = lambda g: [[M(1, g), M(6, g)]]
    outer = lambda g: m16(g) + [[M(7, g), R(0, g)], [R(1, g)]]
    orders = {
        "mid": inner + outer(0) + outer(1),
        "first": [[R(0, 0), R(1, 0)]] + inner + m16(0) + [[M(7, 0)]] + outer(1),
        "last": inner + outer(0) + [[R(1, 1)]] + m16(1) + [[M(7, 1), R(0, 1)]],
    }
    names = ([M(i, 0) for i in LVL1] + [("br", 0)] + [M(i, 1) for i in LVL1] + [("br", 1)]
             + [U(i, u) for i in LVL2 for u in (3, 7)])
    mid_rows = (0, 64, 128, 128, 128, 128, 192, 128, 0, 32, 64, 64, 32, 64, 0, 0)
    rows = {"mid": mid_rows, "last": mid_rows,
            "first": (0, 64, 0, 0, 128, 128, 192, 128, 96, 96, 64, 64, 64, 64, 64, 0)}
    anchors = {}
    for kind, order in orders.items():
        seq = []
        for rnd in order:
            for nm in rnd:
                key = ("br", nm[2]) if nm[0] == "R" else nm
                if key in names and key not in seq:
                    seq.append(key)
        out, tot = {}, 0
        for key in seq:
            n = rows[kind][names.index(key)]
            if not n:
                continue
            nsub = 8 if key[0] == "M" else 4
            steps = n // 8
            pieces = []
            for z in range(nsub):
                take = 8 * (steps // nsub + (1 if z < steps % nsub else 0))
                assert (tot + take - 1) // d == tot // d
                pieces.append((tot // d, take))
                tot += take
            out[key] = pieces
        assert tot == 2 * d
        anchors[kind] = out
    return orders, anchors


def _kernel(x_hbm, g_hbm, b_hbm, w_hbm, o_hbm,
            x_buf, o_buf, w_buf, g_buf, b_buf, a1_sc, a2_sc, ar_sc, t_sc, m_sc, isem, osem):
    S, D, B = x_hbm.shape
    sps = B // SGW
    nsg = S * sps
    orders, anchors = _make_plan(D)

    blocks, g = [], 0
    for n in RAMP + (LOOP_N,) * LOOP_CNT:
        blocks.append((g, n))
        g += n
    assert g == nsg and sum(RAMP) % sps == 0 and LOOP_N % sps == 0
    sets, have = [], 0
    for bi, (g0, n) in enumerate(blocks):
        ahead = 0 if bi == 0 else (sps if g0 % sps == 0 and n % sps == 0 else 1)
        need = min(g0 + n + ahead, nsg)
        sets.append((have, need))
        have = need

    def set_copies(k, merge):
        out, g = [], sets[k][0]
        while g < sets[k][1]:
            s, j = divmod(g, sps)
            if j == 0 and sets[k][1] - g >= sps:
                ns = (sets[k][1] - g) // sps if merge else 1
                idx = (pl.ds(s, ns),)
                g += ns * sps
            else:
                idx = (s, slice(None), pl.ds(j * SGW, SGW))
                g += 1
            out.append(pltpu.make_async_copy(x_hbm.at[idx], x_buf.at[idx], isem.at[k]))
        return out

    param_copies = [pltpu.make_async_copy(src, dst, isem.at[len(sets) + i])
                    for i, (src, dst) in enumerate(((w_hbm, w_buf), (g_hbm, g_buf), (b_hbm, b_buf)))]
    for cp in param_copies:
        cp.start()
    for k in range(len(sets)):
        for cp in set_copies(k, merge=False):
            cp.start()
    for cp in param_copies:
        cp.wait()

    w = w_buf[...]
    row16 = jax.lax.broadcasted_iota(jnp.int32, (16, D), 0)
    b16 = jnp.where(row16 == 0, b_buf[...].astype(F32).reshape(1, D), 0.0).astype(BF16)
    d_row = _dot(b16, w)[0:1, :]
    d_hi = d_row.astype(BF16).astype(F32)
    d_lo = (d_row - d_hi).astype(BF16).astype(F32)
    n_ext = 2 * H + T - D
    row_e = jax.lax.broadcasted_iota(jnp.int32, (n_ext, D), 0)
    ext = jnp.where(row_e == 0, d_hi, jnp.where(row_e == 1, d_lo, 0.0))
    wt = jnp.concatenate([w.astype(F32), ext], axis=0).T
    gf = g_buf[...].astype(F32).reshape(1, D)
    a = wt[:, :2 * H] * gf[:, :2 * H]
    for i in range(1, 8):
        ai = _lin([(sg, a[nh * NH:(nh + 1) * NH, kh * H:(kh + 1) * H]) for sg, nh, kh in A_TERMS[i]])
        if i in LVL1:
            a1_sc[LVL1.index(i)] = pltpu.bitcast(ai.astype(BF16), U32)
        else:
            for u in range(1, 8):
                au = _lin([(sg, ai[nh * NQ:(nh + 1) * NQ, kh * T:(kh + 1) * T]) for sg, nh, kh in A_TERMS[u]])
                a2_sc[LVL2.index(i) * 7 + u - 1] = pltpu.bitcast(au.astype(BF16), U32)
    g_rem = jnp.concatenate([gf[:, 2 * H:], jnp.ones((1, n_ext), F32)], axis=1)
    ar_sc[...] = pltpu.bitcast((wt[:, 2 * H:] * g_rem).astype(BF16), U32)

    class Stats:
        def __init__(self, s, c0):
            self.s, self.cs, self.r = s, slice(c0, c0 + 2 * T), 0

        def piece(self, nrows):
            for r in range(self.r, self.r + nrows, 8):
                x = x_buf[self.s, r:r + 8, self.cs].astype(F32)
                if r == 0:
                    self.c = x[0:1, :]
                y = x - self.c
                self.a1 = y if r == 0 else self.a1 + y
                self.a2 = y * y if r == 0 else self.a2 + y * y
            self.r += nrows
            z = self.a1 + self.a2
            return z[:, :T] + z[:, T:]

        def final(self):
            assert self.r == D
            s1 = jnp.sum(self.a1, axis=0, keepdims=True) * (1.0 / D)
            s2 = jnp.sum(self.a2, axis=0, keepdims=True) * (1.0 / D)
            rs = jax.lax.rsqrt(jnp.maximum(s2 - s1 * s1, 0.0) + EPS)
            return rs, (self.c + s1) * rs

    def super_group(s, c0, st4, nxt, kind, after_half):
        half = lambda v, t: v[:, (t % 2) * T:(t % 2 + 1) * T]
        r = [jnp.broadcast_to(half(st4[2 * (t // 2)], t), (8, T)) for t in range(4)]
        q = [half(st4[2 * (t // 2) + 1], t) for t in range(4)]
        pos = [ri > 0 for ri in r]

        def xblk(r0, nr, t):
            cc = c0 + (t // 2) * 2 * T
            return half(x_buf[s, r0:r0 + nr, cc:cc + 2 * T].astype(F32), t)

        def scale(xs, r8):
            n = xs.shape[0]
            return (xs.reshape(n // 8, 8, T) * r8[None]).reshape(n, T)

        def operand(groups, nr, name):
            tiles = sorted({t for _, t, _ in groups})
            pieces = anchors[kind].get(name) if nxt else None
            parts, const = [], None
            for t in tiles:
                gg = [(sg, inner) for sg, t2, inner in groups if t2 == t]
                xs = _lin([(sg, _lin([(s1, xblk(r0, nr, t)) for s1, r0 in inner])) for sg, inner in gg])
                if pieces is not None and t == tiles[-1]:
                    cr = nr // len(pieces)
                    per = max(1, T // cr)
                    chunks = [None] * len(pieces)
                    korder = sorted(range(len(pieces)), key=lambda k: (-(k % per), -(k // per)))
                    for k, (si, n) in zip(korder, pieces):
                        rr = jnp.where(pos[t], r[t], nxt[si].piece(n)) if n else r[t]
                        chunks[k] = scale(xs[k * cr:(k + 1) * cr], rr)
                    parts.append((1, jnp.concatenate(chunks, axis=0)))
                else:
                    parts.append((1, scale(xs, r[t])))
                net = sum(sg * s1 for sg, inner in gg for s1, _ in inner)
                assert net in (0, 1)
                if net:
                    const = q[t] if const is None else const + q[t]
            val = _lin(parts)
            return (val if const is None else val - const).astype(BF16)

        rem_operand = {}

        def product(name):
            if name[0] == "M":
                _, i, gq = name
                groups = [(sg, 2 * gq + ch, [(1, kh * H)]) for sg, kh, ch in B_TERMS[i]]
                return _dot(pltpu.bitcast(a1_sc[LVL1.index(i)], BF16), operand(groups, H, name))
            if name[0] == "U":
                _, i, u = name
                ch = B_TERMS[i][0][2]
                groups = [(s2, 2 * g2 + ch, [(s1, kh * H + k2 * T) for s1, kh, _ in B_TERMS[i]])
                          for s2, k2, g2 in B_TERMS[u]]
                return _dot(pltpu.bitcast(a2_sc[LVL2.index(i) * 7 + u - 1], BF16), operand(groups, T, name))
            _, nh, gq = name
            if gq not in rem_operand:
                bt = [operand([(1, 2 * gq + ch, [(1, 2 * H)])], D - 2 * H, ("br", gq) if ch == 0 else None)
                      for ch in range(2)]
                ones = jnp.ones((KR - (D - 2 * H), 2 * T), BF16)
                rem_operand[gq] = jnp.concatenate([jnp.concatenate(bt, axis=1), ones], axis=0)
            ar = pltpu.bitcast(ar_sc[nh * NH // 2:(nh + 1) * NH // 2, 0:KR], BF16)
            return _dot(ar, rem_operand[gq])

        m_rem = {(i, nh, g2): set(C_TERMS[(nh, g2)]) for i in LVL2 for nh in range(2) for g2 in range(2)}
        c_rem = {(gq, c): set(C_TERMS[c]) | {"R"} for gq in range(2) for c in C_TERMS}
        m_started, c_started, stored = set(), set(), set()
        t_idx = lambda gq, c: gq * 4 + c[0] * 2 + c[1]
        m_idx = lambda i, gq: LVL2.index(i) * 2 + gq

        for rnd in orders[kind]:
            res = {nm: product(nm) for nm in rnd}
            for key, rem in m_rem.items():
                i, nh, g2 = key
                hit = [nm for nm in rnd if nm[0] == "U" and nm[1] == i and nm[2] in rem]
                if not hit:
                    continue
                terms = [(C_TERMS[(nh, g2)][nm[2]], res[nm]) for nm in hit]
                rem.difference_update(nm[2] for nm in hit)
                if key in m_started:
                    terms.append((2, m_sc[m_idx(i, g2), nh * NQ:(nh + 1) * NQ, :]))
                m_sc[m_idx(i, g2), nh * NQ:(nh + 1) * NQ, :] = _lin(terms)
                m_started.add(key)
            done2 = [{i for i in LVL2 if not m_rem[(i, 0, gq)] and not m_rem[(i, 1, gq)]} for gq in range(2)]
            fresh = {}
            for (gq, c), rem in c_rem.items():
                fresh[(gq, c)] = []
                for nm in rnd:
                    if nm[0] == "M" and nm[2] == gq and nm[1] in rem:
                        fresh[(gq, c)].append((C_TERMS[c][nm[1]], res[nm]))
                        rem.discard(nm[1])
                    if nm[0] == "R" and nm[2] == gq and nm[1] == c[0]:
                        fresh[(gq, c)].append((1, half(res[nm], c[1])))
                        rem.discard("R")
            vals = {}
            for (gq, c), rem in c_rem.items():
                closing = rem <= done2[gq] and c_rem[(gq, (c[0], 1 - c[1]))] <= done2[gq]
                terms = fresh[(gq, c)]
                if not terms and not (rem and closing):
                    continue
                for i in LVL2:
                    if i in rem and i in done2[gq]:
                        terms.append((C_TERMS[c][i], m_sc[m_idx(i, gq)]))
                        rem.discard(i)
                if (gq, c) in c_started:
                    terms.append((2, t_sc[t_idx(gq, c)]))
                c_started.add((gq, c))
                vals[(gq, c)] = _lin(terms)
            for gq in range(2):
                for nh in range(2):
                    if (gq, nh) in stored or c_rem[(gq, (nh, 0))] or c_rem[(gq, (nh, 1))]:
                        continue
                    pair = [vals.pop((gq, (nh, ch))) if (gq, (nh, ch)) in vals else t_sc[t_idx(gq, (nh, ch))]
                            for ch in range(2)]
                    cc = c0 + gq * 2 * T
                    o_buf[s, nh * NH:(nh + 1) * NH, cc:cc + 2 * T] = jnp.concatenate(pair, axis=1).astype(BF16)
                    stored.add((gq, nh))
                    if after_half is not None:
                        after_half(gq, nh)
            for (gq, c), v in vals.items():
                t_sc[t_idx(gq, c)] = v
        assert len(stored) == 4

    def out_copy(*idx):
        return pltpu.make_async_copy(o_buf.at[idx], o_hbm.at[idx], osem)

    def block(s_base, j_base, n, carry, look_ahead=True, it=None):
        for u in range(n):
            ds, j = divmod(j_base + u, sps)
            ds2, j2 = divmod(j_base + u + 1, sps)
            s, s2 = s_base + ds, s_base + ds2
            if u + 1 == n and it is not None:
                s2 = jnp.minimum(s2, S - 1)
            nxt = None
            if look_ahead or u + 1 < n:
                nxt = [Stats(s2, j2 * SGW), Stats(s2, j2 * SGW + 2 * T)]
            kind, after_half = ("first" if u == 0 else "mid"), None
            if it is not None:
                write = pl.when(it >= (W_ITER if ds >= W_SLAB else W_ITER + 1))
                if u == W_SLAB * sps:
                    backlog = (sum(RAMP) + W_ITER * LOOP_N) // sps + W_SLAB
                    pl.when(it == W_ITER)(out_copy(pl.ds(0, backlog)).start)
                if u == n - 1:
                    kind = "last"
                    after_half = lambda gq, nh: write(
                        out_copy(s, pl.ds(nh * NH, NH), pl.ds(j * SGW + gq * 2 * T, 2 * T)).start)
            super_group(s, j * SGW, carry, nxt, kind, after_half)
            if nxt:
                carry = nxt[0].final() + nxt[1].final()
            if it is not None and u < n - 1:
                if u >= n - sps:
                    write(out_copy(s, slice(None), pl.ds(j * SGW, SGW)).start)
                elif j == sps - 1:
                    write(out_copy(s).start)
        return carry

    def full_stats(g0):
        out = ()
        for gq in range(2):
            st = Stats(g0 // sps, (g0 % sps) * SGW + gq * 2 * T)
            st.piece(D)
            out += st.final()
        return out

    carry = None
    for bi in range(len(RAMP)):
        g0, n = blocks[bi]
        for cp in set_copies(bi, merge=True):
            cp.wait()
        if bi < 2:
            carry = full_stats(g0)
        carry = block(g0 // sps, g0 % sps, n, carry, look_ahead=bi > 0)
    k0 = len(RAMP)
    for cp in set_copies(k0, merge=True):
        cp.wait()
    ns = LOOP_N // sps

    def body(it, carry):
        sb = sum(RAMP) // sps + it * ns
        carry = block(sb, 0, LOOP_N, carry, it=it)

        def wait_next(n_slabs):
            pltpu.make_async_copy(x_hbm.at[pl.ds(0, n_slabs)], x_buf.at[pl.ds(sb + ns + 1, n_slabs)],
                                  isem.at[k0 + 1 + it]).wait()

        pl.when(it < LOOP_CNT - 2)(lambda: wait_next(ns))
        pl.when(it == LOOP_CNT - 2)(lambda: wait_next(ns - 1))
        return carry

    jax.lax.fori_loop(0, LOOP_CNT, body, carry)
    pltpu.make_async_copy(o_buf, o_hbm, osem).wait()


@jax.jit
def pallas_standalone__layernorm_linear__sampling_kernel(
    x: jax.Array,
    g: jax.Array,
    b: jax.Array,
    w: jax.Array,
):
    B, S, D = x.shape
    xt = jnp.transpose(x, (1, 2, 0))
    out_t = pl.pallas_call(
        _kernel,
        in_specs=[pl.BlockSpec(memory_space=pl.ANY)] * 4,
        out_specs=pl.BlockSpec(memory_space=pl.ANY),
        out_shape=jax.ShapeDtypeStruct((S, D, B), x.dtype),
        scratch_shapes=[
            pltpu.VMEM((S, D, B), BF16),
            pltpu.VMEM((S, D, B), BF16),
            pltpu.VMEM((D, D), BF16),
            pltpu.VMEM((D,), BF16),
            pltpu.VMEM((D,), BF16),
            pltpu.VMEM((len(LVL1), NH // 2, H), U32),
            pltpu.VMEM((7 * len(LVL2), NQ // 2, T), U32),
            pltpu.VMEM((NH, T), U32),
            pltpu.VMEM((8, NH, T), F32),
            pltpu.VMEM((2 * len(LVL2), NH, T), F32),
            pltpu.SemaphoreType.DMA((len(RAMP) + LOOP_CNT + 3,)),
            pltpu.SemaphoreType.DMA(()),
        ],
        compiler_params=pltpu.CompilerParams(
            vmem_limit_bytes=110 * 1024 * 1024,
            disable_bounds_checks=True,
        ),
    )(xt, g, b, w)
    return jnp.transpose(out_t, (2, 0, 1))
```

```python
import jax
import jax.numpy as jnp
import jax.experimental.pallas as pl
import jax.experimental.pallas.tpu as pltpu

EPS = 1e-5
F32 = jnp.float32
BF16 = jnp.bfloat16
U32 = jnp.uint32

T = 128
H = 256
NH = 288
NQ = 144
KR = 80
SGW = 512

B_TERMS = {1: ((1, 0, 0), (1, 1, 1)), 2: ((1, 0, 0),), 3: ((1, 0, 1), (-1, 1, 1)), 4: ((1, 1, 0), (-1, 0, 0)),
           5: ((1, 1, 1),), 6: ((1, 0, 0), (1, 0, 1)), 7: ((1, 1, 0), (1, 1, 1))}
A_TERMS = {1: ((1, 0, 0), (1, 1, 1)), 2: ((1, 1, 0), (1, 1, 1)), 3: ((1, 0, 0),), 4: ((1, 1, 1),),
           5: ((1, 0, 0), (1, 0, 1)), 6: ((1, 1, 0), (-1, 0, 0)), 7: ((1, 0, 1), (-1, 1, 1))}
C_TERMS = {(0, 0): {1: 1, 4: 1, 5: -1, 7: 1}, (0, 1): {3: 1, 5: 1},
           (1, 0): {2: 1, 4: 1}, (1, 1): {1: 1, 2: -1, 3: 1, 6: 1}}

LVL2 = (2, 5, 3, 4)
LVL1 = (1, 6, 7)

RAMP = (1, 1, 2, 4)
LOOP_N, LOOP_CNT = 8, 7
W_ITER, W_SLAB = 2, 2


def _dot(a, b):
    return jnp.dot(a, b, preferred_element_type=F32)


def _lin(terms):
    terms = sorted(terms, key=lambda t: -t[0])
    assert terms[0][0] > 0
    acc = terms[0][1]
    for sg, v in terms[1:]:
        acc = acc + v if sg > 0 else acc - v
    return acc


def _make_plan(d):
    M = lambda i, g: ("M", i, g)
    U = lambda i, u: ("U", i, u)
    R = lambda nh, g: ("R", nh, g)
    inner = []
    for i in LVL2:
        inner += [[U(i, 1), U(i, 4), U(i, 5), U(i, 3)], [U(i, 2), U(i, 6), U(i, 7)]]
    m16 = lambda g: [[M(1, g), M(6, g)]]
    outer = lambda g: m16(g) + [[M(7, g), R(0, g)], [R(1, g)]]
    orders = {
        "mid": inner + outer(0) + outer(1),
        "first": [[R(0, 0), R(1, 0)]] + inner + m16(0) + [[M(7, 0)]] + outer(1),
        "last": inner + outer(0) + [[R(1, 1)]] + m16(1) + [[M(7, 1), R(0, 1)]],
    }
    names = ([M(i, 0) for i in LVL1] + [("br", 0)] + [M(i, 1) for i in LVL1] + [("br", 1)]
             + [U(i, u) for i in LVL2 for u in (3, 7)])
    mid_rows = (0, 64, 128, 128, 128, 128, 192, 128, 0, 32, 64, 64, 32, 64, 0, 0)
    rows = {"mid": mid_rows, "last": mid_rows,
            "first": (0, 64, 0, 0, 128, 128, 192, 128, 96, 96, 64, 64, 64, 64, 64, 0)}
    anchors = {}
    for kind, order in orders.items():
        seq = []
        for rnd in order:
            for nm in rnd:
                key = ("br", nm[2]) if nm[0] == "R" else nm
                if key in names and key not in seq:
                    seq.append(key)
        out, tot = {}, 0
        for key in seq:
            n = rows[kind][names.index(key)]
            if not n:
                continue
            nsub = 8 if key[0] == "M" else 4
            steps = n // 8
            pieces = []
            for z in range(nsub):
                take = 8 * (steps // nsub + (1 if z < steps % nsub else 0))
                assert (tot + take - 1) // d == tot // d
                pieces.append((tot // d, take))
                tot += take
            out[key] = pieces
        assert tot == 2 * d
        anchors[kind] = out
    return orders, anchors


def _kernel(x_hbm, g_hbm, b_hbm, w_hbm, o_hbm,
            x_buf, o_buf, w_buf, g_buf, b_buf, a1_sc, a2_sc, ar_sc, t_sc, m_sc, isem, osem):
    S, D, B = x_hbm.shape
    sps = B // SGW
    nsg = S * sps
    orders, anchors = _make_plan(D)

    blocks, g = [], 0
    for n in RAMP + (LOOP_N,) * LOOP_CNT:
        blocks.append((g, n))
        g += n
    assert g == nsg and sum(RAMP) % sps == 0 and LOOP_N % sps == 0
    sets, have = [], 0
    for bi, (g0, n) in enumerate(blocks):
        ahead = 0 if bi == 0 else (sps if g0 % sps == 0 and n % sps == 0 else 1)
        need = min(g0 + n + ahead, nsg)
        sets.append((have, need))
        have = need

    def set_copies(k):
        out, g = [], sets[k][0]
        while g < sets[k][1]:
            s, j = divmod(g, sps)
            if j == 0 and sets[k][1] - g >= sps:
                ns = (sets[k][1] - g) // sps if k >= len(RAMP) else 1
                idx = (pl.ds(s, ns),)
                g += ns * sps
            else:
                idx = (s, slice(None), pl.ds(j * SGW, SGW))
                g += 1
            out.append(pltpu.make_async_copy(x_hbm.at[idx], x_buf.at[idx], isem.at[k]))
        return out

    param_copies = [pltpu.make_async_copy(src, dst, isem.at[len(sets) + i])
                    for i, (src, dst) in enumerate(((w_hbm, w_buf), (g_hbm, g_buf), (b_hbm, b_buf)))]
    for cp in param_copies:
        cp.start()
    for k in range(len(sets)):
        for cp in set_copies(k):
            cp.start()
    for cp in param_copies:
        cp.wait()

    w = w_buf[...]
    row16 = jax.lax.broadcasted_iota(jnp.int32, (16, D), 0)
    b16 = jnp.where(row16 == 0, b_buf[...].astype(F32).reshape(1, D), 0.0).astype(BF16)
    d_row = _dot(b16, w)[0:1, :]
    d_hi = d_row.astype(BF16).astype(F32)
    d_lo = (d_row - d_hi).astype(BF16).astype(F32)
    n_ext = 2 * H + T - D
    row_e = jax.lax.broadcasted_iota(jnp.int32, (n_ext, D), 0)
    ext = jnp.where(row_e == 0, d_hi, jnp.where(row_e == 1, d_lo, 0.0))
    wt = jnp.concatenate([w.astype(F32), ext], axis=0).T
    gf = g_buf[...].astype(F32).reshape(1, D)
    a = wt[:, :2 * H] * gf[:, :2 * H]
    for i in range(1, 8):
        ai = _lin([(sg, a[nh * NH:(nh + 1) * NH, kh * H:(kh + 1) * H]) for sg, nh, kh in A_TERMS[i]])
        if i in LVL1:
            a1_sc[LVL1.index(i)] = pltpu.bitcast(ai.astype(BF16), U32)
        else:
            for u in range(1, 8):
                au = _lin([(sg, ai[nh * NQ:(nh + 1) * NQ, kh * T:(kh + 1) * T]) for sg, nh, kh in A_TERMS[u]])
                a2_sc[LVL2.index(i) * 7 + u - 1] = pltpu.bitcast(au.astype(BF16), U32)
    g_rem = jnp.concatenate([gf[:, 2 * H:], jnp.ones((1, n_ext), F32)], axis=1)
    ar_sc[...] = pltpu.bitcast((wt[:, 2 * H:] * g_rem).astype(BF16), U32)

    class Stats:
        def __init__(self, s, c0):
            self.s, self.cs, self.r = s, slice(c0, c0 + 2 * T), 0

        def piece(self, nrows):
            for r in range(self.r, self.r + nrows, 8):
                x = x_buf[self.s, r:r + 8, self.cs].astype(F32)
                if r == 0:
                    self.c = x[0:1, :]
                y = x - self.c
                self.a1 = y if r == 0 else self.a1 + y
                self.a2 = y * y if r == 0 else self.a2 + y * y
            self.r += nrows
            z = self.a1 + self.a2
            return z[:, :T] + z[:, T:]

        def final(self):
            assert self.r == D
            s1 = jnp.sum(self.a1, axis=0, keepdims=True) * (1.0 / D)
            s2 = jnp.sum(self.a2, axis=0, keepdims=True) * (1.0 / D)
            rs = jax.lax.rsqrt(jnp.maximum(s2 - s1 * s1, 0.0) + EPS)
            return rs, (self.c + s1) * rs

    def super_group(s, c0, st4, nxt, kind, after_half):
        half = lambda v, t: v[:, (t % 2) * T:(t % 2 + 1) * T]
        r = [jnp.broadcast_to(half(st4[2 * (t // 2)], t), (8, T)) for t in range(4)]
        q = [half(st4[2 * (t // 2) + 1], t) for t in range(4)]
        pos = [ri > 0 for ri in r]

        def xblk(r0, nr, t):
            cc = c0 + (t // 2) * 2 * T
            return half(x_buf[s, r0:r0 + nr, cc:cc + 2 * T].astype(F32), t)

        def scale(xs, r8):
            n = xs.shape[0]
            return (xs.reshape(n // 8, 8, T) * r8[None]).reshape(n, T)

        def operand(groups, nr, name):
            tiles = sorted({t for _, t, _ in groups})
            pieces = anchors[kind].get(name) if nxt else None
            parts, const = [], None
            for t in tiles:
                gg = [(sg, inner) for sg, t2, inner in groups if t2 == t]
                xs = _lin([(sg, _lin([(s1, xblk(r0, nr, t)) for s1, r0 in inner])) for sg, inner in gg])
                if pieces is not None and t == tiles[-1]:
                    cr = nr // len(pieces)
                    per = max(1, T // cr)
                    chunks = [None] * len(pieces)
                    korder = sorted(range(len(pieces)), key=lambda k: (-(k % per), -(k // per)))
                    for k, (si, n) in zip(korder, pieces):
                        rr = jnp.where(pos[t], r[t], nxt[si].piece(n)) if n else r[t]
                        chunks[k] = scale(xs[k * cr:(k + 1) * cr], rr)
                    parts.append((1, jnp.concatenate(chunks, axis=0)))
                else:
                    parts.append((1, scale(xs, r[t])))
                net = sum(sg * s1 for sg, inner in gg for s1, _ in inner)
                assert net in (0, 1)
                if net:
                    const = q[t] if const is None else const + q[t]
            val = _lin(parts)
            return (val if const is None else val - const).astype(BF16)

        rem_operand = {}

        def product(name):
            if name[0] == "M":
                _, i, gq = name
                groups = [(sg, 2 * gq + ch, [(1, kh * H)]) for sg, kh, ch in B_TERMS[i]]
                return _dot(pltpu.bitcast(a1_sc[LVL1.index(i)], BF16), operand(groups, H, name))
            if name[0] == "U":
                _, i, u = name
                ch = B_TERMS[i][0][2]
                groups = [(s2, 2 * g2 + ch, [(s1, kh * H + k2 * T) for s1, kh, _ in B_TERMS[i]])
                          for s2, k2, g2 in B_TERMS[u]]
                return _dot(pltpu.bitcast(a2_sc[LVL2.index(i) * 7 + u - 1], BF16), operand(groups, T, name))
            _, nh, gq = name
            if gq not in rem_operand:
                bt = [operand([(1, 2 * gq + ch, [(1, 2 * H)])], D - 2 * H, ("br", gq) if ch == 0 else None)
                      for ch in range(2)]
                ones = jnp.ones((KR - (D - 2 * H), 2 * T), BF16)
                rem_operand[gq] = jnp.concatenate([jnp.concatenate(bt, axis=1), ones], axis=0)
            ar = pltpu.bitcast(ar_sc[nh * NH // 2:(nh + 1) * NH // 2, 0:KR], BF16)
            return _dot(ar, rem_operand[gq])

        m_rem = {(i, nh, g2): set(C_TERMS[(nh, g2)]) for i in LVL2 for nh in range(2) for g2 in range(2)}
        c_rem = {(gq, c): set(C_TERMS[c]) | {"R"} for gq in range(2) for c in C_TERMS}
        m_started, c_started, stored = set(), set(), set()
        t_idx = lambda gq, c: gq * 4 + c[0] * 2 + c[1]
        m_idx = lambda i, gq: LVL2.index(i) * 2 + gq

        for rnd in orders[kind]:
            res = {nm: product(nm) for nm in rnd}
            for key, rem in m_rem.items():
                i, nh, g2 = key
                hit = [nm for nm in rnd if nm[0] == "U" and nm[1] == i and nm[2] in rem]
                if not hit:
                    continue
                terms = [(C_TERMS[(nh, g2)][nm[2]], res[nm]) for nm in hit]
                rem.difference_update(nm[2] for nm in hit)
                if key in m_started:
                    terms.append((2, m_sc[m_idx(i, g2), nh * NQ:(nh + 1) * NQ, :]))
                m_sc[m_idx(i, g2), nh * NQ:(nh + 1) * NQ, :] = _lin(terms)
                m_started.add(key)
            done2 = [{i for i in LVL2 if not m_rem[(i, 0, gq)] and not m_rem[(i, 1, gq)]} for gq in range(2)]
            fresh = {}
            for (gq, c), rem in c_rem.items():
                fresh[(gq, c)] = []
                for nm in rnd:
                    if nm[0] == "M" and nm[2] == gq and nm[1] in rem:
                        fresh[(gq, c)].append((C_TERMS[c][nm[1]], res[nm]))
                        rem.discard(nm[1])
                    if nm[0] == "R" and nm[2] == gq and nm[1] == c[0]:
                        fresh[(gq, c)].append((1, half(res[nm], c[1])))
                        rem.discard("R")
            vals = {}
            for (gq, c), rem in c_rem.items():
                closing = rem <= done2[gq] and c_rem[(gq, (c[0], 1 - c[1]))] <= done2[gq]
                terms = fresh[(gq, c)]
                if not terms and not (rem and closing):
                    continue
                for i in LVL2:
                    if i in rem and i in done2[gq]:
                        terms.append((C_TERMS[c][i], m_sc[m_idx(i, gq)]))
                        rem.discard(i)
                if (gq, c) in c_started:
                    terms.append((2, t_sc[t_idx(gq, c)]))
                c_started.add((gq, c))
                vals[(gq, c)] = _lin(terms)
            for gq in range(2):
                for nh in range(2):
                    if (gq, nh) in stored or c_rem[(gq, (nh, 0))] or c_rem[(gq, (nh, 1))]:
                        continue
                    pair = [vals.pop((gq, (nh, ch))) if (gq, (nh, ch)) in vals else t_sc[t_idx(gq, (nh, ch))]
                            for ch in range(2)]
                    cc = c0 + gq * 2 * T
                    o_buf[s, nh * NH:(nh + 1) * NH, cc:cc + 2 * T] = jnp.concatenate(pair, axis=1).astype(BF16)
                    stored.add((gq, nh))
                    if after_half is not None:
                        after_half(gq, nh)
            for (gq, c), v in vals.items():
                t_sc[t_idx(gq, c)] = v
        assert len(stored) == 4

    def out_copy(*idx):
        return pltpu.make_async_copy(o_buf.at[idx], o_hbm.at[idx], osem)

    def block(s_base, j_base, n, carry, look_ahead=True, it=None):
        for u in range(n):
            ds, j = divmod(j_base + u, sps)
            ds2, j2 = divmod(j_base + u + 1, sps)
            s, s2 = s_base + ds, s_base + ds2
            if u + 1 == n and it is not None:
                s2 = jnp.minimum(s2, S - 1)
            nxt = None
            if look_ahead or u + 1 < n:
                nxt = [Stats(s2, j2 * SGW), Stats(s2, j2 * SGW + 2 * T)]
            kind, after_half = ("first" if u == 0 else "mid"), None
            if it is not None:
                write = pl.when(it >= (W_ITER if ds >= W_SLAB else W_ITER + 1))
                if u == W_SLAB * sps:
                    backlog = (sum(RAMP) + W_ITER * LOOP_N) // sps + W_SLAB
                    pl.when(it == W_ITER)(out_copy(pl.ds(0, backlog)).start)
                if u == n - 1:
                    kind = "last"
                    after_half = lambda gq, nh: write(
                        out_copy(s, pl.ds(nh * NH, NH), pl.ds(j * SGW + gq * 2 * T, 2 * T)).start)
            super_group(s, j * SGW, carry, nxt, kind, after_half)
            if nxt:
                carry = nxt[0].final() + nxt[1].final()
            if it is not None and u < n - 1:
                if u >= n - sps:
                    write(out_copy(s, slice(None), pl.ds(j * SGW, SGW)).start)
                elif j == sps - 1:
                    write(out_copy(s).start)
        return carry

    def full_stats(g0):
        out = ()
        for gq in range(2):
            st = Stats(g0 // sps, (g0 % sps) * SGW + gq * 2 * T)
            st.piece(D)
            out += st.final()
        return out

    carry = None
    for bi in range(len(RAMP)):
        g0, n = blocks[bi]
        for cp in set_copies(bi):
            cp.wait()
        if bi < 2:
            carry = full_stats(g0)
        carry = block(g0 // sps, g0 % sps, n, carry, look_ahead=bi > 0)
    k0 = len(RAMP)
    for cp in set_copies(k0):
        cp.wait()
    ns = LOOP_N // sps

    def body(it, carry):
        sb = sum(RAMP) // sps + it * ns
        carry = block(sb, 0, LOOP_N, carry, it=it)

        def wait_next(n_slabs):
            slabs = pl.ds(sb + ns + 1, n_slabs)
            pltpu.make_async_copy(x_hbm.at[slabs], x_buf.at[slabs], isem.at[k0 + 1 + it]).wait()

        pl.when(it < LOOP_CNT - 2)(lambda: wait_next(ns))
        pl.when(it == LOOP_CNT - 2)(lambda: wait_next(ns - 1))
        return carry

    jax.lax.fori_loop(0, LOOP_CNT, body, carry)
    pltpu.make_async_copy(o_buf, o_hbm, osem).wait()


@jax.jit
def pallas_standalone__layernorm_linear__sampling_kernel(
    x: jax.Array,
    g: jax.Array,
    b: jax.Array,
    w: jax.Array,
):
    B, S, D = x.shape
    xt = jnp.transpose(x, (1, 2, 0))
    no_checks = {name: True for name in ("disable_bounds_checks", "disable_semaphore_checks")
                 if hasattr(pltpu.CompilerParams, name)}
    out_t = pl.pallas_call(
        _kernel,
        in_specs=[pl.BlockSpec(memory_space=pl.ANY)] * 4,
        out_specs=pl.BlockSpec(memory_space=pl.ANY),
        out_shape=jax.ShapeDtypeStruct((S, D, B), x.dtype),
        scratch_shapes=[
            pltpu.VMEM((S, D, B), BF16),
            pltpu.VMEM((S, D, B), BF16),
            pltpu.VMEM((D, D), BF16),
            pltpu.VMEM((D,), BF16),
            pltpu.VMEM((D,), BF16),
            pltpu.VMEM((len(LVL1), NH // 2, H), U32),
            pltpu.VMEM((7 * len(LVL2), NQ // 2, T), U32),
            pltpu.VMEM((NH, T), U32),
            pltpu.VMEM((8, NH, T), F32),
            pltpu.VMEM((2 * len(LVL2), NH, T), F32),
            pltpu.SemaphoreType.DMA((len(RAMP) + LOOP_CNT + 3,)),
            pltpu.SemaphoreType.DMA(()),
        ],
        compiler_params=pltpu.CompilerParams(vmem_limit_bytes=110 * 1024 * 1024, **no_checks),
    )(xt, g, b, w)
    return jnp.transpose(out_t, (2, 0, 1))
```

```python
import jax
import jax.numpy as jnp
import jax.experimental.pallas as pl
import jax.experimental.pallas.tpu as pltpu

EPS = 1e-5
F32 = jnp.float32
BF16 = jnp.bfloat16
U32 = jnp.uint32

T = 128
H = 256
NH = 288
NQ = 144
KR = 80
SGW = 512

B_TERMS = {1: ((1, 0, 0), (1, 1, 1)), 2: ((1, 0, 0),), 3: ((1, 0, 1), (-1, 1, 1)), 4: ((1, 1, 0), (-1, 0, 0)),
           5: ((1, 1, 1),), 6: ((1, 0, 0), (1, 0, 1)), 7: ((1, 1, 0), (1, 1, 1))}
A_TERMS = {1: ((1, 0, 0), (1, 1, 1)), 2: ((1, 1, 0), (1, 1, 1)), 3: ((1, 0, 0),), 4: ((1, 1, 1),),
           5: ((1, 0, 0), (1, 0, 1)), 6: ((1, 1, 0), (-1, 0, 0)), 7: ((1, 0, 1), (-1, 1, 1))}
C_TERMS = {(0, 0): {1: 1, 4: 1, 5: -1, 7: 1}, (0, 1): {3: 1, 5: 1},
           (1, 0): {2: 1, 4: 1}, (1, 1): {1: 1, 2: -1, 3: 1, 6: 1}}

LVL2 = (2, 5, 3, 4)
LVL1 = (1, 6, 7)
SWAP = (3, 4)

RAMP = (1, 1, 2, 4)
LOOP_N, LOOP_CNT = 8, 7
W_ITER, W_SLAB = 2, 2


def _dot(a, b):
    return jnp.dot(a, b, preferred_element_type=F32)


def _lin(terms):
    terms = sorted(terms, key=lambda t: -t[0])
    assert terms[0][0] > 0
    acc = terms[0][1]
    for sg, v in terms[1:]:
        acc = acc + v if sg > 0 else acc - v
    return acc


def _make_plan(d):
    M = lambda i, g: ("M", i, g)
    U = lambda i, u: ("U", i, u)
    R = lambda nh, g: ("R", nh, g)
    inner = []
    for i in LVL2:
        inner += [[U(i, 1), U(i, 4), U(i, 5), U(i, 3)], [U(i, 2), U(i, 6), U(i, 7)]]
    m16 = lambda g: [[M(1, g), M(6, g)]]
    outer = lambda g: m16(g) + [[M(7, g), R(0, g)], [R(1, g)]]
    orders = {
        "mid": inner + outer(0) + outer(1),
        "first": [[R(0, 0), R(1, 0)]] + inner + m16(0) + [[M(7, 0)]] + outer(1),
        "last": inner + outer(0) + [[R(1, 1)]] + m16(1) + [[M(7, 1), R(0, 1)]],
    }
    names = ([M(i, 0) for i in LVL1] + [("br", 0)] + [M(i, 1) for i in LVL1] + [("br", 1)]
             + [U(i, u) for i in LVL2 for u in (3, 7)])
    mid_rows = (0, 64, 128, 128, 128, 128, 192, 128, 0, 32, 64, 64, 32, 64, 0, 0)
    rows = {"mid": mid_rows, "last": mid_rows,
            "first": (0, 64, 0, 0, 128, 128, 192, 128, 96, 96, 64, 64, 64, 64, 64, 0)}
    anchors = {}
    for kind, order in orders.items():
        seq = []
        for rnd in order:
            for nm in rnd:
                key = ("br", nm[2]) if nm[0] == "R" else nm
                if key in names and key not in seq:
                    seq.append(key)
        out, tot = {}, 0
        for key in seq:
            n = rows[kind][names.index(key)]
            if not n:
                continue
            nsub = 8 if key[0] == "M" else 4
            steps = n // 8
            pieces = []
            for z in range(nsub):
                take = 8 * (steps // nsub + (1 if z < steps % nsub else 0))
                assert (tot + take - 1) // d == tot // d
                pieces.append((tot // d, take))
                tot += take
            out[key] = pieces
        assert tot == 2 * d
        anchors[kind] = out
    return orders, anchors


def _kernel(x_hbm, g_hbm, b_hbm, w_hbm, o_hbm,
            x_buf, o_buf, w_buf, g_buf, b_buf, a1_sc, a2_sc, ar_sc, t_sc, m_sc, isem, osem):
    S, D, B = x_hbm.shape
    sps = B // SGW
    nsg = S * sps
    orders, anchors = _make_plan(D)

    blocks, g = [], 0
    for n in RAMP + (LOOP_N,) * LOOP_CNT:
        blocks.append((g, n))
        g += n
    assert g == nsg and sum(RAMP) % sps == 0 and LOOP_N % sps == 0
    sets, have = [], 0
    for bi, (g0, n) in enumerate(blocks):
        ahead = 0 if bi == 0 else (sps if g0 % sps == 0 and n % sps == 0 else 1)
        need = min(g0 + n + ahead, nsg)
        sets.append((have, need))
        have = need

    def set_copies(k):
        out, g = [], sets[k][0]
        while g < sets[k][1]:
            s, j = divmod(g, sps)
            if j == 0 and sets[k][1] - g >= sps:
                ns = (sets[k][1] - g) // sps if k >= len(RAMP) else 1
                idx = (pl.ds(s, ns),)
                g += ns * sps
            else:
                idx = (s, slice(None), pl.ds(j * SGW, SGW))
                g += 1
            out.append(pltpu.make_async_copy(x_hbm.at[idx], x_buf.at[idx], isem.at[k]))
        return out

    param_copies = [pltpu.make_async_copy(src, dst, isem.at[len(sets) + i])
                    for i, (src, dst) in enumerate(((w_hbm, w_buf), (g_hbm, g_buf), (b_hbm, b_buf)))]
    for cp in param_copies:
        cp.start()
    for k in range(len(sets)):
        for cp in set_copies(k):
            cp.start()
    for cp in param_copies:
        cp.wait()

    w = w_buf[...]
    row16 = jax.lax.broadcasted_iota(jnp.int32, (16, D), 0)
    b16 = jnp.where(row16 == 0, b_buf[...].astype(F32).reshape(1, D), 0.0).astype(BF16)
    d_row = _dot(b16, w)[0:1, :]
    d_hi = d_row.astype(BF16).astype(F32)
    d_lo = (d_row - d_hi).astype(BF16).astype(F32)
    n_ext = 2 * H + T - D
    row_e = jax.lax.broadcasted_iota(jnp.int32, (n_ext, D), 0)
    ext = jnp.where(row_e == 0, d_hi, jnp.where(row_e == 1, d_lo, 0.0))
    wt = jnp.concatenate([w.astype(F32), ext], axis=0).T
    gf = g_buf[...].astype(F32).reshape(1, D)
    a = wt[:, :2 * H] * gf[:, :2 * H]
    for i in range(1, 8):
        ai = _lin([(sg, a[nh * NH:(nh + 1) * NH, kh * H:(kh + 1) * H]) for sg, nh, kh in A_TERMS[i]])
        if i in LVL1:
            a1_sc[LVL1.index(i)] = pltpu.bitcast(ai.astype(BF16), U32)
        else:
            for u in range(1, 8):
                au = _lin([(sg, ai[nh * NQ:(nh + 1) * NQ, kh * T:(kh + 1) * T]) for sg, nh, kh in A_TERMS[u]])
                a2_sc[LVL2.index(i) * 7 + u - 1] = pltpu.bitcast(au.astype(BF16), U32)
    g_rem = jnp.concatenate([gf[:, 2 * H:], jnp.ones((1, n_ext), F32)], axis=1)
    ar_sc[...] = pltpu.bitcast((wt[:, 2 * H:] * g_rem).astype(BF16), U32)

    class Stats:
        def __init__(self, s, c0):
            self.s, self.cs, self.r = s, slice(c0, c0 + 2 * T), 0

        def piece(self, nrows):
            for r in range(self.r, self.r + nrows, 8):
                x = x_buf[self.s, r:r + 8, self.cs].astype(F32)
                if r == 0:
                    self.c = x[0:1, :]
                y = x - self.c
                self.a1 = y if r == 0 else self.a1 + y
                self.a2 = y * y if r == 0 else self.a2 + y * y
            self.r += nrows
            z = self.a1 + self.a2
            return z[:, :T] + z[:, T:]

        def final(self):
            assert self.r == D
            s1 = jnp.sum(self.a1, axis=0, keepdims=True) * (1.0 / D)
            s2 = jnp.sum(self.a2, axis=0, keepdims=True) * (1.0 / D)
            rs = jax.lax.rsqrt(jnp.maximum(s2 - s1 * s1, 0.0) + EPS)
            return rs, (self.c + s1) * rs

    def super_group(s, c0, st4, nxt, kind, after_half):
        half = lambda v, t: v[:, (t % 2) * T:(t % 2 + 1) * T]
        r = [jnp.broadcast_to(half(st4[2 * (t // 2)], t), (8, T)) for t in range(4)]
        q = [half(st4[2 * (t // 2) + 1], t) for t in range(4)]
        pos = [ri > 0 for ri in r]

        def xblk(r0, nr, t):
            cc = c0 + (t // 2) * 2 * T
            return half(x_buf[s, r0:r0 + nr, cc:cc + 2 * T].astype(F32), t)

        def scale(xs, r8):
            n = xs.shape[0]
            return (xs.reshape(n // 8, 8, T) * r8[None]).reshape(n, T)

        def operand(groups, nr, name):
            tiles = sorted({t for _, t, _ in groups})
            pieces = anchors[kind].get(name) if nxt else None
            parts, const = [], None
            for t in tiles:
                gg = [(sg, inner) for sg, t2, inner in groups if t2 == t]
                xs = _lin([(sg, _lin([(s1, xblk(r0, nr, t)) for s1, r0 in inner])) for sg, inner in gg])
                if pieces is not None and t == tiles[-1]:
                    cr = nr // len(pieces)
                    per = max(1, T // cr)
                    chunks = [None] * len(pieces)
                    korder = sorted(range(len(pieces)), key=lambda k: (-(k % per), -(k // per)))
                    for k, (si, n) in zip(korder, pieces):
                        rr = jnp.where(pos[t], r[t], nxt[si].piece(n)) if n else r[t]
                        chunks[k] = scale(xs[k * cr:(k + 1) * cr], rr)
                    parts.append((1, jnp.concatenate(chunks, axis=0)))
                else:
                    parts.append((1, scale(xs, r[t])))
                net = sum(sg * s1 for sg, inner in gg for s1, _ in inner)
                assert net in (0, 1)
                if net:
                    const = q[t] if const is None else const + q[t]
            val = _lin(parts)
            return (val if const is None else val - const).astype(BF16)

        rem_operand = {}

        def product(name):
            if name[0] == "M":
                _, i, gq = name
                groups = [(sg, 2 * gq + ch, [(1, kh * H)]) for sg, kh, ch in B_TERMS[i]]
                return _dot(pltpu.bitcast(a1_sc[LVL1.index(i)], BF16), operand(groups, H, name))
            if name[0] == "U":
                _, i, u = name
                ch = B_TERMS[i][0][2]
                groups = [(s2, 2 * (g2 ^ (i in SWAP)) + ch, [(s1, kh * H + k2 * T) for s1, kh, _ in B_TERMS[i]])
                          for s2, k2, g2 in B_TERMS[u]]
                return _dot(pltpu.bitcast(a2_sc[LVL2.index(i) * 7 + u - 1], BF16), operand(groups, T, name))
            _, nh, gq = name
            if gq not in rem_operand:
                bt = [operand([(1, 2 * gq + ch, [(1, 2 * H)])], D - 2 * H, ("br", gq) if ch == 0 else None)
                      for ch in range(2)]
                ones = jnp.ones((KR - (D - 2 * H), 2 * T), BF16)
                rem_operand[gq] = jnp.concatenate([jnp.concatenate(bt, axis=1), ones], axis=0)
            ar = pltpu.bitcast(ar_sc[nh * NH // 2:(nh + 1) * NH // 2, 0:KR], BF16)
            return _dot(ar, rem_operand[gq])

        m_terms = lambda i, nh, gq: C_TERMS[(nh, gq ^ (i in SWAP))]
        m_rem = {(i, nh, g2): set(m_terms(i, nh, g2)) for i in LVL2 for nh in range(2) for g2 in range(2)}
        c_rem = {(gq, c): set(C_TERMS[c]) | {"R"} for gq in range(2) for c in C_TERMS}
        m_started, c_started, stored = set(), set(), set()
        t_idx = lambda gq, c: gq * 4 + c[0] * 2 + c[1]
        m_idx = lambda i, gq: LVL2.index(i) * 2 + gq

        for rnd in orders[kind]:
            res = {nm: product(nm) for nm in rnd}
            for key, rem in m_rem.items():
                i, nh, g2 = key
                hit = [nm for nm in rnd if nm[0] == "U" and nm[1] == i and nm[2] in rem]
                if not hit:
                    continue
                terms = [(m_terms(i, nh, g2)[nm[2]], res[nm]) for nm in hit]
                rem.difference_update(nm[2] for nm in hit)
                if key in m_started:
                    terms.append((2, m_sc[m_idx(i, g2), nh * NQ:(nh + 1) * NQ, :]))
                m_sc[m_idx(i, g2), nh * NQ:(nh + 1) * NQ, :] = _lin(terms)
                m_started.add(key)
            done2 = [{i for i in LVL2 if not m_rem[(i, 0, gq)] and not m_rem[(i, 1, gq)]} for gq in range(2)]
            fresh = {}
            for (gq, c), rem in c_rem.items():
                fresh[(gq, c)] = []
                for nm in rnd:
                    if nm[0] == "M" and nm[2] == gq and nm[1] in rem:
                        fresh[(gq, c)].append((C_TERMS[c][nm[1]], res[nm]))
                        rem.discard(nm[1])
                    if nm[0] == "R" and nm[2] == gq and nm[1] == c[0]:
                        fresh[(gq, c)].append((1, half(res[nm], c[1])))
                        rem.discard("R")
            vals = {}
            for (gq, c), rem in c_rem.items():
                closing = rem <= done2[gq] and c_rem[(gq, (c[0], 1 - c[1]))] <= done2[gq]
                terms = fresh[(gq, c)]
                if not terms and not (rem and closing):
                    continue
                for i in LVL2:
                    if i in rem and i in done2[gq]:
                        terms.append((C_TERMS[c][i], m_sc[m_idx(i, gq)]))
                        rem.discard(i)
                if (gq, c) in c_started:
                    terms.append((2, t_sc[t_idx(gq, c)]))
                c_started.add((gq, c))
                vals[(gq, c)] = _lin(terms)
            for gq in range(2):
                for nh in range(2):
                    if (gq, nh) in stored or c_rem[(gq, (nh, 0))] or c_rem[(gq, (nh, 1))]:
                        continue
                    pair = [vals.pop((gq, (nh, ch))) if (gq, (nh, ch)) in vals else t_sc[t_idx(gq, (nh, ch))]
                            for ch in range(2)]
                    cc = c0 + gq * 2 * T
                    o_buf[s, nh * NH:(nh + 1) * NH, cc:cc + 2 * T] = jnp.concatenate(pair, axis=1).astype(BF16)
                    stored.add((gq, nh))
                    if after_half is not None:
                        after_half(gq, nh)
            for (gq, c), v in vals.items():
                t_sc[t_idx(gq, c)] = v
        assert len(stored) == 4

    def out_copy(*idx):
        return pltpu.make_async_copy(o_buf.at[idx], o_hbm.at[idx], osem)

    def block(s_base, j_base, n, carry, look_ahead=True, it=None):
        for u in range(n):
            ds, j = divmod(j_base + u, sps)
            ds2, j2 = divmod(j_base + u + 1, sps)
            s, s2 = s_base + ds, s_base + ds2
            if u + 1 == n and it is not None:
                s2 = jnp.minimum(s2, S - 1)
            nxt = None
            if look_ahead or u + 1 < n:
                nxt = [Stats(s2, j2 * SGW), Stats(s2, j2 * SGW + 2 * T)]
            kind, after_half = ("first" if u == 0 else "mid"), None
            if it is not None:
                write = pl.when(it >= (W_ITER if ds >= W_SLAB else W_ITER + 1))
                if u == W_SLAB * sps:
                    backlog = (sum(RAMP) + W_ITER * LOOP_N) // sps + W_SLAB
                    pl.when(it == W_ITER)(out_copy(pl.ds(0, backlog)).start)
                if u == n - 1:
                    kind = "last"
                    after_half = lambda gq, nh: write(
                        out_copy(s, pl.ds(nh * NH, NH), pl.ds(j * SGW + gq * 2 * T, 2 * T)).start)
            super_group(s, j * SGW, carry, nxt, kind, after_half)
            if nxt:
                carry = nxt[0].final() + nxt[1].final()
            if it is not None and u < n - 1:
                if u >= n - sps:
                    write(out_copy(s, slice(None), pl.ds(j * SGW, SGW)).start)
                elif j == sps - 1:
                    write(out_copy(s).start)
        return carry

    def full_stats(g0):
        out = ()
        for gq in range(2):
            st = Stats(g0 // sps, (g0 % sps) * SGW + gq * 2 * T)
            st.piece(D)
            out += st.final()
        return out

    carry = None
    for bi in range(len(RAMP)):
        g0, n = blocks[bi]
        for cp in set_copies(bi):
            cp.wait()
        if bi < 2:
            carry = full_stats(g0)
        carry = block(g0 // sps, g0 % sps, n, carry, look_ahead=bi > 0)
    k0 = len(RAMP)
    for cp in set_copies(k0):
        cp.wait()
    ns = LOOP_N // sps

    def body(it, carry):
        sb = sum(RAMP) // sps + it * ns
        carry = block(sb, 0, LOOP_N, carry, it=it)

        def wait_next(n_slabs):
            slabs = pl.ds(sb + ns + 1, n_slabs)
            pltpu.make_async_copy(x_hbm.at[slabs], x_buf.at[slabs], isem.at[k0 + 1 + it]).wait()

        pl.when(it < LOOP_CNT - 2)(lambda: wait_next(ns))
        pl.when(it == LOOP_CNT - 2)(lambda: wait_next(ns - 1))
        return carry

    jax.lax.fori_loop(0, LOOP_CNT, body, carry)
    pltpu.make_async_copy(o_buf, o_hbm, osem).wait()


@jax.jit
def pallas_standalone__layernorm_linear__sampling_kernel(
    x: jax.Array,
    g: jax.Array,
    b: jax.Array,
    w: jax.Array,
):
    B, S, D = x.shape
    xt = jnp.transpose(x, (1, 2, 0))
    no_checks = {name: True for name in ("disable_bounds_checks", "disable_semaphore_checks")
                 if hasattr(pltpu.CompilerParams, name)}
    out_t = pl.pallas_call(
        _kernel,
        in_specs=[pl.BlockSpec(memory_space=pl.ANY)] * 4,
        out_specs=pl.BlockSpec(memory_space=pl.ANY),
        out_shape=jax.ShapeDtypeStruct((S, D, B), x.dtype),
        scratch_shapes=[
            pltpu.VMEM((S, D, B), BF16),
            pltpu.VMEM((S, D, B), BF16),
            pltpu.VMEM((D, D), BF16),
            pltpu.VMEM((D,), BF16),
            pltpu.VMEM((D,), BF16),
            pltpu.VMEM((len(LVL1), NH // 2, H), U32),
            pltpu.VMEM((7 * len(LVL2), NQ // 2, T), U32),
            pltpu.VMEM((NH, T), U32),
            pltpu.VMEM((8, NH, T), F32),
            pltpu.VMEM((2 * len(LVL2), NH, T), F32),
            pltpu.SemaphoreType.DMA((len(RAMP) + LOOP_CNT + 3,)),
            pltpu.SemaphoreType.DMA(()),
        ],
        compiler_params=pltpu.CompilerParams(vmem_limit_bytes=110 * 1024 * 1024, **no_checks),
    )(xt, g, b, w)
    return jnp.transpose(out_t, (2, 0, 1))
```

```python
import jax
import jax.numpy as jnp
import jax.experimental.pallas as pl
import jax.experimental.pallas.tpu as pltpu

EPS = 1e-5
F32 = jnp.float32
BF16 = jnp.bfloat16
U32 = jnp.uint32

T = 128
H = 256
NH = 288
NQ = 144
KR = 80
SGW = 512

B_TERMS = {1: ((1, 0, 0), (1, 1, 1)), 2: ((1, 0, 0),), 3: ((1, 0, 1), (-1, 1, 1)), 4: ((1, 1, 0), (-1, 0, 0)),
           5: ((1, 1, 1),), 6: ((1, 0, 0), (1, 0, 1)), 7: ((1, 1, 0), (1, 1, 1))}
A_TERMS = {1: ((1, 0, 0), (1, 1, 1)), 2: ((1, 1, 0), (1, 1, 1)), 3: ((1, 0, 0),), 4: ((1, 1, 1),),
           5: ((1, 0, 0), (1, 0, 1)), 6: ((1, 1, 0), (-1, 0, 0)), 7: ((1, 0, 1), (-1, 1, 1))}
C_TERMS = {(0, 0): {1: 1, 4: 1, 5: -1, 7: 1}, (0, 1): {3: 1, 5: 1},
           (1, 0): {2: 1, 4: 1}, (1, 1): {1: 1, 2: -1, 3: 1, 6: 1}}

OUTER = (2, 5, 3, 4, 1, 6, 7)
INNER = ((1, 4, 5, 3), (2, 6, 7))
SWAP = (3, 4, 6, 7)
N_EARLY = 2

RAMP = (1, 1, 2, 4)
LOOP_N, LOOP_CNT = 8, 7
W_ITER, W_POS = 2, 2
W_ROWS = 32


def _dot(a, b):
    return jnp.dot(a, b, preferred_element_type=F32)


def _lin(terms):
    terms = sorted(terms, key=lambda t: -t[0])
    assert terms[0][0] > 0
    acc = terms[0][1]
    for sg, v in terms[1:]:
        acc = acc + v if sg > 0 else acc - v
    return acc


def _make_plan(d, last):
    rounds = [[(i, u) for u in us] for i in OUTER for us in INNER]
    if last:
        rounds = rounds[:-2] + [[("R", 1, 0)], [("R", 1, 1)]] + rounds[-2:] + [[("R", 0, 0)], [("R", 0, 1)]]
    else:
        rounds += [[("R", nh, gq)] for gq in range(2) for nh in range(2)]
    slots = []
    for rnd in rounds:
        for nm in rnd:
            if nm[0] == "R":
                key, wt = ("R", nm[2]), 3.0
            else:
                pos = OUTER.index(nm[0])
                key, wt = nm, (1.3 if pos >= 4 else float(pos > 0 and nm[1] in INNER[1]))
            if all(key != k for k, _ in slots):
                slots += [(key, wt)] * 2
    steps = d // 8
    scale = 2 * steps / sum(wt for _, wt in slots)
    pieces, acc, done = {}, 0.0, 0
    for key, wt in slots:
        acc += wt * scale
        take = int(round(acc)) - done
        if done < steps:
            take = min(take, steps - done)
        pieces.setdefault(key, []).append((min(done // steps, 1), 8 * take))
        done += take
    assert done == 2 * steps
    return rounds, pieces


def _kernel(x_hbm, g_hbm, b_hbm, w_hbm, o_hbm,
            x_buf, o_buf, w_buf, g_buf, b_buf, a_sc, ar_sc, m_sc, xn_sc, isem, osem):
    S, D, B = x_hbm.shape
    sps = B // SGW
    nsg = S * sps
    plans = {last: _make_plan(D, last) for last in (False, True)}

    blocks, g = [], 0
    for n in RAMP + (LOOP_N,) * LOOP_CNT:
        blocks.append((g, n))
        g += n
    assert g == nsg and sum(RAMP) % sps == 0 and LOOP_N == 4 * sps == 8
    sets, have = [], 0
    for bi, (g0, n) in enumerate(blocks):
        need = min(g0 + n + (bi > 0), nsg)
        sets.append((have, need))
        have = need

    def x_copy(idx, sem):
        return pltpu.make_async_copy(x_hbm.at[idx], x_buf.at[idx], isem.at[sem])

    def set_copies(k, shift=0, sem=None):
        out, g = [], sets[k][0]
        while g < sets[k][1]:
            s, j = divmod(g, sps)
            if j == 0 and sets[k][1] - g >= sps:
                ns = (sets[k][1] - g) // sps if k >= len(RAMP) else 1
                out.append(x_copy((pl.ds(s + shift, ns),), k if sem is None else sem))
                g += ns * sps
            else:
                out.append(x_copy((s + shift, slice(None), pl.ds(j * SGW, SGW)), k if sem is None else sem))
                g += 1
        return out

    def first_copies():
        return [x_copy((0, slice(None), pl.ds(gq * 2 * T, 2 * T)), (len(sets), 0)[gq]) for gq in range(2)]

    param_copies = [pltpu.make_async_copy(src, dst, isem.at[len(sets) + 1 + i])
                    for i, (src, dst) in enumerate(((w_hbm, w_buf), (g_hbm, g_buf), (b_hbm, b_buf)))]
    for cp in param_copies + first_copies():
        cp.start()
    for k in range(1, len(sets)):
        for cp in set_copies(k):
            cp.start()
    for cp in param_copies:
        cp.wait()

    w = w_buf[...]
    row16 = jax.lax.broadcasted_iota(jnp.int32, (16, D), 0)
    b16 = jnp.where(row16 == 0, b_buf[...].astype(F32).reshape(1, D), 0.0).astype(BF16)
    d_row = _dot(b16, w)[0:1, :]
    d_hi = d_row.astype(BF16).astype(F32)
    d_lo = (d_row - d_hi).astype(BF16).astype(F32)
    n_ext = 2 * H + T - D
    row_e = jax.lax.broadcasted_iota(jnp.int32, (n_ext, D), 0)
    ext = jnp.where(row_e == 0, d_hi, jnp.where(row_e == 1, d_lo, 0.0))
    wt = jnp.concatenate([w.astype(F32), ext], axis=0).T
    gf = g_buf[...].astype(F32).reshape(1, D)
    a = wt[:, :2 * H] * gf[:, :2 * H]
    a_idx = lambda i, u: OUTER.index(i) * 7 + u - 1

    def prep_left(i):
        ai = _lin([(sg, a[nh * NH:(nh + 1) * NH, kh * H:(kh + 1) * H]) for sg, nh, kh in A_TERMS[i]])
        for u in range(1, 8):
            au = _lin([(sg, ai[nh * NQ:(nh + 1) * NQ, kh * T:(kh + 1) * T]) for sg, nh, kh in A_TERMS[u]])
            a_sc[a_idx(i, u)] = pltpu.bitcast(au.astype(BF16), U32)

    for i in OUTER[:N_EARLY]:
        prep_left(i)
    g_rem = jnp.concatenate([gf[:, 2 * H:], jnp.ones((1, n_ext), F32)], axis=1)
    ar_sc[...] = pltpu.bitcast((wt[:, 2 * H:] * g_rem).astype(BF16), U32)

    class Stats:
        def __init__(self, s, c0):
            self.s, self.cs, self.r = s, slice(c0, c0 + 2 * T), 0

        def piece(self, nrows):
            for r in range(self.r, self.r + nrows, 8):
                x = x_buf[self.s, r:r + 8, self.cs].astype(F32)
                if r == 0:
                    self.c = x[0:1, :]
                y = x - self.c
                self.a1 = y if r == 0 else self.a1 + y
                self.a2 = y * y if r == 0 else self.a2 + y * y
            self.r += nrows
            z = self.a1 + self.a2
            return z[:, :T] + z[:, T:]

        def final(self):
            assert self.r == D
            s1 = jnp.sum(self.a1, axis=0, keepdims=True) * (1.0 / D)
            s2 = jnp.sum(self.a2, axis=0, keepdims=True) * (1.0 / D)
            rs = jax.lax.rsqrt(jnp.maximum(s2 - s1 * s1, 0.0) + EPS)
            return rs, (self.c + s1) * rs

        def whole(self):
            self.piece(D)
            return self.final()

    def super_group(s, c0, slot, st4, nxt, after_half):
        rounds, pieces = plans[after_half is not None]
        half = lambda v, t: v[:, (t % 2) * T:(t % 2 + 1) * T]
        r = [jnp.broadcast_to(half(st4[2 * (t // 2)], t), (8, T)) for t in range(4)]
        q = [half(st4[2 * (t // 2) + 1], t) for t in range(4)]
        always = r[0] > 0

        def normalised(r0, nr, t):
            cc = c0 + (t // 2) * 2 * T
            x = half(x_buf[s, r0:r0 + nr, cc:cc + 2 * T].astype(F32), t)
            return (x.reshape(nr // 8, 8, T) * r[t][None]).reshape(nr, T) - q[t]

        in_round, in_mem = {}, set()

        def xhat(kb, t):
            if (kb, t) not in in_round:
                if (kb, t) in in_mem:
                    in_round[(kb, t)] = xn_sc[slot, kb * 4 + t]
                else:
                    in_round[(kb, t)] = normalised(kb * T, T, t)
                    xn_sc[slot, kb * 4 + t] = in_round[(kb, t)]
                    in_mem.add((kb, t))
            return in_round[(kb, t)]

        def rounded(val, key):
            if nxt is not None:
                cr = val.shape[0] // 2
                segs = []
                for k in (1, 0):
                    si, n = pieces[key][1 - k]
                    lo = (k + 1) * cr - 8
                    tied = jnp.where(always, val[lo:lo + 8], nxt[si].piece(n)) if n else val[lo:lo + 8]
                    segs = [val[k * cr:lo], tied] + segs
                if any(n for _, n in pieces[key]):
                    val = jnp.concatenate(segs, axis=0)
            return val.astype(BF16)

        rem_operand = {}
        m_idx = lambda i, gq: OUTER.index(i) * 2 + gq
        for rnd in rounds:
            in_round.clear()
            if rnd[0][0] == "R":
                _, nh, gq = rnd[0]
                if gq not in rem_operand:
                    bt = [normalised(2 * H, D - 2 * H, 2 * gq + ch) for ch in range(2)]
                    bt = jnp.concatenate([rounded(bt[0], ("R", gq)), bt[1].astype(BF16)], axis=1)
                    ones = jnp.ones((KR - (D - 2 * H), 2 * T), BF16)
                    rem_operand[gq] = jnp.concatenate([bt, ones], axis=0)
                ar = pltpu.bitcast(ar_sc[nh * NH // 2:(nh + 1) * NH // 2, 0:KR], BF16)
                res = _dot(ar, rem_operand[gq])
                pair = [_lin([(1, half(res, ch))] + [(C_TERMS[(nh, ch)][i], m_sc[m_idx(i, gq)])
                                                     for i in OUTER if i in C_TERMS[(nh, ch)]])
                        for ch in range(2)]
                cc = c0 + gq * 2 * T
                o_buf[2 * s + nh, :, cc:cc + 2 * T] = jnp.concatenate(pair, axis=1).astype(BF16)
                if after_half is not None:
                    after_half(gq, nh)
                continue
            i = rnd[0][0]
            sw = int(i in SWAP)
            res = {}
            for _, u in rnd:
                val = _lin([(s2, _lin([(s1, xhat(2 * kh + k2, 2 * (g2 ^ sw) + ch)) for s1, kh, ch in B_TERMS[i]]))
                            for s2, k2, g2 in B_TERMS[u]])
                res[u] = _dot(pltpu.bitcast(a_sc[a_idx(i, u)], BF16), rounded(val, (i, u)))
            for nh in range(2):
                for gq in range(2):
                    ct = C_TERMS[(nh, gq ^ sw)]
                    terms = [(ct[u], res[u]) for _, u in rnd if u in ct]
                    if not terms:
                        continue
                    if rnd[0][1] != INNER[0][0]:
                        terms.append((2, m_sc[m_idx(i, gq), nh * NQ:(nh + 1) * NQ, :]))
                    m_sc[m_idx(i, gq), nh * NQ:(nh + 1) * NQ, :] = _lin(terms)

    def out_copy(*idx):
        return pltpu.make_async_copy(o_buf.at[idx], o_hbm.at[idx], osem)

    def write_slabs(cond, s0, n):
        for r in range(0, NH, W_ROWS):
            pl.when(cond)(out_copy(pl.ds(2 * s0, 2 * n), pl.ds(r, W_ROWS)).start)

    def block(s_base, j_base, n, carry, look_ahead=True, it=None):
        for u in range(n):
            ds, j = divmod(j_base + u, sps)
            ds2, j2 = divmod(j_base + u + 1, sps)
            s, s2 = s_base + ds, s_base + ds2
            if u + 1 == n and it is not None:
                s2 = jnp.minimum(s2, S - 1)
            nxt = None
            if look_ahead or u + 1 < n:
                nxt = [Stats(s2, j2 * SGW), Stats(s2, j2 * SGW + 2 * T)]
            after_half = None
            if it is not None:
                final = it == LOOP_CNT - 1
                steady = jnp.logical_and(it >= W_ITER, it < LOOP_CNT - 1)
                if 0 <= u - W_POS < W_ITER + 1:
                    write_slabs(it == W_ITER, 4 * (u - W_POS), 4)
                if u == n - 1:
                    after_half = lambda gq, nh: pl.when(final)(
                        out_copy(2 * s + nh, slice(None), pl.ds(j * SGW + gq * 2 * T, 2 * T)).start)
            super_group(s, j * SGW, u, carry, nxt, after_half)
            if nxt is not None:
                carry = nxt[0].final() + nxt[1].final()
            if it is not None:
                if u in (1, 3, 5):
                    write_slabs(final, s, 1)
                if u in (3, 7):
                    write_slabs(steady, s - 1, 2)
                if u == 6:
                    for gq in range(2):
                        pl.when(final)(out_copy(pl.ds(2 * s, 2), slice(None), pl.ds(gq * 2 * T, 2 * T)).start)
        return carry

    assert sum(RAMP) == LOOP_N and W_POS <= 3 and W_POS + W_ITER < LOOP_N
    carry = ()
    for gq, cp in enumerate(first_copies()):
        cp.wait()
        carry += Stats(0, gq * 2 * T).whole()
    for i in OUTER[N_EARLY:]:
        prep_left(i)
    for bi in range(len(RAMP)):
        g0, n = blocks[bi]
        if bi == 1:
            carry = sum((Stats(g0 // sps, (g0 % sps) * SGW + gq * 2 * T).whole() for gq in range(2)), ())
        carry = block(g0 // sps, g0 % sps, n, carry, look_ahead=bi > 0)
        for cp in set_copies(bi + 1):
            cp.wait()
    k0, ns = len(RAMP), LOOP_N // sps

    def body(it, carry):
        carry = block(sum(RAMP) // sps + it * ns, 0, LOOP_N, carry, it=it)

        @pl.when(it < LOOP_CNT - 2)
        def _():
            for cp in set_copies(k0 + 1, shift=it * ns, sem=k0 + 1 + it):
                cp.wait()

        @pl.when(it == LOOP_CNT - 2)
        def _():
            for cp in set_copies(k0 + LOOP_CNT - 1):
                cp.wait()

        return carry

    jax.lax.fori_loop(0, LOOP_CNT, body, carry)
    pltpu.make_async_copy(o_buf, o_hbm, osem).wait()


@jax.jit
def pallas_standalone__layernorm_linear__sampling_kernel(
    x: jax.Array,
    g: jax.Array,
    b: jax.Array,
    w: jax.Array,
):
    B, S, D = x.shape
    xt = jnp.transpose(x, (1, 2, 0))
    no_checks = {name: True for name in ("disable_bounds_checks", "disable_semaphore_checks")
                 if hasattr(pltpu.CompilerParams, name)}
    out_t = pl.pallas_call(
        _kernel,
        in_specs=[pl.BlockSpec(memory_space=pl.ANY)] * 4,
        out_specs=pl.BlockSpec(memory_space=pl.ANY),
        out_shape=jax.ShapeDtypeStruct((2 * S, NH, B), x.dtype),
        scratch_shapes=[
            pltpu.VMEM((S, D, B), BF16),
            pltpu.VMEM((2 * S, NH, B), BF16),
            pltpu.VMEM((D, D), BF16),
            pltpu.VMEM((D,), BF16),
            pltpu.VMEM((D,), BF16),
            pltpu.VMEM((49, NQ // 2, T), U32),
            pltpu.VMEM((NH, T), U32),
            pltpu.VMEM((14, NH, T), F32),
            pltpu.VMEM((LOOP_N, 16, T, T), F32),
            pltpu.SemaphoreType.DMA((len(RAMP) + LOOP_CNT + 4,)),
            pltpu.SemaphoreType.DMA(()),
        ],
        compiler_params=pltpu.CompilerParams(vmem_limit_bytes=110 * 1024 * 1024, **no_checks),
    )(xt, g, b, w)
    return jnp.transpose(out_t.reshape(S, D, B), (2, 0, 1))
```

```python
import jax
import jax.numpy as jnp
import jax.experimental.pallas as pl
import jax.experimental.pallas.tpu as pltpu

EPS = 1e-5
F32 = jnp.float32
BF16 = jnp.bfloat16
U32 = jnp.uint32

T = 128
H = 256
NH = 288
NQ = 144
KR = 80
SGW = 512

B_TERMS = {1: ((1, 0, 0), (1, 1, 1)), 2: ((1, 0, 0),), 3: ((1, 0, 1), (1, 1, 1)), 4: ((1, 1, 0), (1, 0, 0)),
           5: ((1, 1, 1),), 6: ((1, 0, 0), (-1, 0, 1)), 7: ((1, 1, 0), (-1, 1, 1))}
A_TERMS = {1: ((1, 0, 0), (-1, 1, 1)), 2: ((1, 1, 0), (-1, 1, 1)), 3: ((1, 0, 0),), 4: ((1, 1, 1),),
           5: ((1, 0, 0), (-1, 0, 1)), 6: ((1, 1, 0), (-1, 0, 0)), 7: ((1, 0, 1), (-1, 1, 1))}
C_TERMS = {(0, 0): {1: 1, 4: 1, 5: -1, 7: 1}, (0, 1): {3: 1, 5: -1},
           (1, 0): {2: 1, 4: 1}, (1, 1): {1: -1, 2: 1, 3: 1, 6: -1}}

OUTER = (2, 5, 3, 4, 1, 6, 7)
INNER = ((1, 4, 5, 3), (2, 6, 7))
SWAP = (3, 4, 6, 7)
N_EARLY = 2

RAMP = (1, 1, 2, 4)
LOOP_N, LOOP_CNT = 8, 7
W_ITER, W_POS = 2, 2
W_ROWS = 32


def _dot(a, b):
    return jnp.dot(a, b, preferred_element_type=F32)


def _lin(terms):
    terms = sorted(terms, key=lambda t: -t[0])
    assert terms[0][0] > 0
    acc = terms[0][1]
    for sg, v in terms[1:]:
        acc = acc + v if sg > 0 else acc - v
    return acc


def _make_plan(d, last):
    rounds = [[(i, u) for u in us] for i in OUTER for us in INNER]
    if last:
        rounds = rounds[:-2] + [[("R", 1, 0)], [("R", 1, 1)]] + rounds[-2:] + [[("R", 0, 0)], [("R", 0, 1)]]
    else:
        rounds += [[("R", nh, gq)] for gq in range(2) for nh in range(2)]
    slots = []
    for rnd in rounds:
        for nm in rnd:
            if nm[0] == "R":
                key, wt = ("R", nm[2]), 3.0
            else:
                pos = OUTER.index(nm[0])
                key, wt = nm, (1.3 if pos >= 4 else float(pos > 0 and nm[1] in INNER[1]))
            if all(key != k for k, _ in slots):
                slots += [(key, wt)] * 2
    steps = d // 8
    scale = 2 * steps / sum(wt for _, wt in slots)
    pieces, acc, done = {}, 0.0, 0
    for key, wt in slots:
        acc += wt * scale
        take = int(round(acc)) - done
        if done < steps:
            take = min(take, steps - done)
        pieces.setdefault(key, []).append((min(done // steps, 1), 8 * take))
        done += take
    assert done == 2 * steps
    return rounds, pieces


def _kernel(x_hbm, g_hbm, b_hbm, w_hbm, o_hbm,
            x_buf, o_buf, w_buf, g_buf, b_buf, a_sc, ar_sc, m_sc, xn_sc, isem, osem):
    S, D, B = x_hbm.shape
    sps = B // SGW
    nsg = S * sps
    plans = {last: _make_plan(D, last) for last in (False, True)}

    blocks, g = [], 0
    for n in RAMP + (LOOP_N,) * LOOP_CNT:
        blocks.append((g, n))
        g += n
    assert g == nsg and sum(RAMP) % sps == 0 and LOOP_N == 4 * sps == 8
    sets, have = [], 0
    for bi, (g0, n) in enumerate(blocks):
        need = min(g0 + n + (bi > 0), nsg)
        sets.append((have, need))
        have = need

    def x_copy(idx, sem):
        return pltpu.make_async_copy(x_hbm.at[idx], x_buf.at[idx], isem.at[sem])

    def set_copies(k, shift=0, sem=None):
        out, g = [], sets[k][0]
        while g < sets[k][1]:
            s, j = divmod(g, sps)
            if j == 0 and sets[k][1] - g >= sps:
                ns = (sets[k][1] - g) // sps if k >= len(RAMP) else 1
                out.append(x_copy((pl.ds(s + shift, ns),), k if sem is None else sem))
                g += ns * sps
            else:
                out.append(x_copy((s + shift, slice(None), pl.ds(j * SGW, SGW)), k if sem is None else sem))
                g += 1
        return out

    def first_copies():
        return [x_copy((0, slice(None), pl.ds(gq * 2 * T, 2 * T)), (len(sets), 0)[gq]) for gq in range(2)]

    param_copies = [pltpu.make_async_copy(src, dst, isem.at[len(sets) + 1 + i])
                    for i, (src, dst) in enumerate(((w_hbm, w_buf), (g_hbm, g_buf), (b_hbm, b_buf)))]
    for cp in param_copies + first_copies():
        cp.start()
    for k in range(1, len(sets)):
        for cp in set_copies(k):
            cp.start()
    for cp in param_copies:
        cp.wait()

    w = w_buf[...]
    row16 = jax.lax.broadcasted_iota(jnp.int32, (16, D), 0)
    b16 = jnp.where(row16 == 0, b_buf[...].astype(F32).reshape(1, D), 0.0).astype(BF16)
    d_row = _dot(b16, w)[0:1, :]
    d_hi = d_row.astype(BF16).astype(F32)
    d_lo = (d_row - d_hi).astype(BF16).astype(F32)
    n_ext = 2 * H + T - D
    row_e = jax.lax.broadcasted_iota(jnp.int32, (n_ext, D), 0)
    ext = jnp.where(row_e == 0, d_hi, jnp.where(row_e == 1, d_lo, 0.0))
    wt = jnp.concatenate([w.astype(F32), ext], axis=0).T
    gf = g_buf[...].astype(F32).reshape(1, D)
    a = wt[:, :2 * H] * gf[:, :2 * H]
    a_idx = lambda i, u: OUTER.index(i) * 7 + u - 1

    def prep_left(i):
        ai = _lin([(sg, a[nh * NH:(nh + 1) * NH, kh * H:(kh + 1) * H]) for sg, nh, kh in A_TERMS[i]])
        for u in range(1, 8):
            au = _lin([(sg, ai[nh * NQ:(nh + 1) * NQ, kh * T:(kh + 1) * T]) for sg, nh, kh in A_TERMS[u]])
            a_sc[a_idx(i, u)] = pltpu.bitcast(au.astype(BF16), U32)

    for i in OUTER[:N_EARLY]:
        prep_left(i)
    g_rem = jnp.concatenate([gf[:, 2 * H:], jnp.ones((1, n_ext), F32)], axis=1)
    ar_sc[...] = pltpu.bitcast((wt[:, 2 * H:] * g_rem).astype(BF16), U32)

    class Stats:
        def __init__(self, s, c0):
            self.s, self.cs, self.r = s, slice(c0, c0 + 2 * T), 0

        def piece(self, nrows):
            for r in range(self.r, self.r + nrows, 8):
                x = x_buf[self.s, r:r + 8, self.cs].astype(F32)
                if r == 0:
                    self.c = x[0:1, :]
                y = x - self.c
                self.a1 = y if r == 0 else self.a1 + y
                self.a2 = y * y if r == 0 else self.a2 + y * y
            self.r += nrows
            z = self.a1 + self.a2
            return z[:, :T] + z[:, T:]

        def final(self):
            assert self.r == D
            s1 = jnp.sum(self.a1, axis=0, keepdims=True) * (1.0 / D)
            s2 = jnp.sum(self.a2, axis=0, keepdims=True) * (1.0 / D)
            rs = jax.lax.rsqrt(jnp.maximum(s2 - s1 * s1, 0.0) + EPS)
            return rs, (self.c + s1) * rs

        def whole(self):
            self.piece(D)
            return self.final()

    def super_group(s, c0, slot, st4, nxt, after_half):
        rounds, pieces = plans[after_half is not None]
        half = lambda v, t: v[:, (t % 2) * T:(t % 2 + 1) * T]
        r = [jnp.broadcast_to(half(st4[2 * (t // 2)], t), (8, T)) for t in range(4)]
        q = [half(st4[2 * (t // 2) + 1], t) for t in range(4)]
        always = r[0] > 0

        def normalised(r0, nr, t):
            cc = c0 + (t // 2) * 2 * T
            x = half(x_buf[s, r0:r0 + nr, cc:cc + 2 * T].astype(F32), t)
            return (x.reshape(nr // 8, 8, T) * r[t][None]).reshape(nr, T) - q[t]

        in_round, in_mem = {}, set()

        def xhat(kb, t):
            if (kb, t) not in in_round:
                if (kb, t) in in_mem:
                    in_round[(kb, t)] = xn_sc[slot, kb * 4 + t]
                else:
                    in_round[(kb, t)] = normalised(kb * T, T, t)
                    xn_sc[slot, kb * 4 + t] = in_round[(kb, t)]
                    in_mem.add((kb, t))
            return in_round[(kb, t)]

        def rounded(val, key):
            if nxt is not None:
                cr = val.shape[0] // 2
                segs = []
                for k in (1, 0):
                    si, n = pieces[key][1 - k]
                    lo = (k + 1) * cr - 8
                    tied = jnp.where(always, val[lo:lo + 8], nxt[si].piece(n)) if n else val[lo:lo + 8]
                    segs = [val[k * cr:lo], tied] + segs
                if any(n for _, n in pieces[key]):
                    val = jnp.concatenate(segs, axis=0)
            return val.astype(BF16)

        rem_operand = {}
        m_idx = lambda i, gq: OUTER.index(i) * 2 + gq
        for rnd in rounds:
            in_round.clear()
            if rnd[0][0] == "R":
                _, nh, gq = rnd[0]
                if gq not in rem_operand:
                    bt = [normalised(2 * H, D - 2 * H, 2 * gq + ch) for ch in range(2)]
                    bt = jnp.concatenate([rounded(bt[0], ("R", gq)), bt[1].astype(BF16)], axis=1)
                    ones = jnp.ones((KR - (D - 2 * H), 2 * T), BF16)
                    rem_operand[gq] = jnp.concatenate([bt, ones], axis=0)
                ar = pltpu.bitcast(ar_sc[nh * NH // 2:(nh + 1) * NH // 2, 0:KR], BF16)
                res = _dot(ar, rem_operand[gq])
                pair = [_lin([(1, half(res, ch))] + [(C_TERMS[(nh, ch)][i], m_sc[m_idx(i, gq)])
                                                     for i in OUTER if i in C_TERMS[(nh, ch)]])
                        for ch in range(2)]
                cc = c0 + gq * 2 * T
                o_buf[2 * s + nh, :, cc:cc + 2 * T] = jnp.concatenate(pair, axis=1).astype(BF16)
                if after_half is not None:
                    after_half(gq, nh)
                continue
            i = rnd[0][0]
            sw = int(i in SWAP)
            res = {}
            for _, u in rnd:
                val = _lin([(s2, _lin([(s1, xhat(2 * kh + k2, 2 * (g2 ^ sw) + ch)) for s1, kh, ch in B_TERMS[i]]))
                            for s2, k2, g2 in B_TERMS[u]])
                res[u] = _dot(pltpu.bitcast(a_sc[a_idx(i, u)], BF16), rounded(val, (i, u)))
            for nh in range(2):
                for gq in range(2):
                    ct = C_TERMS[(nh, gq ^ sw)]
                    terms = [(ct[u], res[u]) for _, u in rnd if u in ct]
                    if not terms:
                        continue
                    if rnd[0][1] != INNER[0][0]:
                        terms.append((2, m_sc[m_idx(i, gq), nh * NQ:(nh + 1) * NQ, :]))
                    m_sc[m_idx(i, gq), nh * NQ:(nh + 1) * NQ, :] = _lin(terms)

    def out_copy(*idx):
        return pltpu.make_async_copy(o_buf.at[idx], o_hbm.at[idx], osem)

    def write_slabs(cond, s0, n):
        for r in range(0, NH, W_ROWS):
            pl.when(cond)(out_copy(pl.ds(2 * s0, 2 * n), pl.ds(r, W_ROWS)).start)

    def block(s_base, j_base, n, carry, look_ahead=True, it=None):
        for u in range(n):
            ds, j = divmod(j_base + u, sps)
            ds2, j2 = divmod(j_base + u + 1, sps)
            s, s2 = s_base + ds, s_base + ds2
            if u + 1 == n and it is not None:
                s2 = jnp.minimum(s2, S - 1)
            nxt = None
            if look_ahead or u + 1 < n:
                nxt = [Stats(s2, j2 * SGW), Stats(s2, j2 * SGW + 2 * T)]
            after_half = None
            if it is not None:
                final = it == LOOP_CNT - 1
                steady = jnp.logical_and(it >= W_ITER, it < LOOP_CNT - 1)
                if 0 <= u - W_POS < W_ITER + 1:
                    write_slabs(it == W_ITER, 4 * (u - W_POS), 4)
                if u == n - 1:
                    after_half = lambda gq, nh: pl.when(final)(
                        out_copy(2 * s + nh, slice(None), pl.ds(j * SGW + gq * 2 * T, 2 * T)).start)
            super_group(s, j * SGW, u, carry, nxt, after_half)
            if nxt is not None:
                carry = nxt[0].final() + nxt[1].final()
            if it is not None:
                if u in (1, 3, 5):
                    write_slabs(final, s, 1)
                if u in (3, 7):
                    write_slabs(steady, s - 1, 2)
                if u == 6:
                    for gq in range(2):
                        pl.when(final)(out_copy(pl.ds(2 * s, 2), slice(None), pl.ds(gq * 2 * T, 2 * T)).start)
        return carry

    assert sum(RAMP) == LOOP_N and W_POS <= 3 and W_POS + W_ITER < LOOP_N
    carry = ()
    for gq, cp in enumerate(first_copies()):
        cp.wait()
        carry += Stats(0, gq * 2 * T).whole()
    for i in OUTER[N_EARLY:]:
        prep_left(i)
    for bi in range(len(RAMP)):
        g0, n = blocks[bi]
        if bi == 1:
            carry = sum((Stats(g0 // sps, (g0 % sps) * SGW + gq * 2 * T).whole() for gq in range(2)), ())
        carry = block(g0 // sps, g0 % sps, n, carry, look_ahead=bi > 0)
        for cp in set_copies(bi + 1):
            cp.wait()
    k0, ns = len(RAMP), LOOP_N // sps

    def body(it, carry):
        carry = block(sum(RAMP) // sps + it * ns, 0, LOOP_N, carry, it=it)

        @pl.when(it < LOOP_CNT - 2)
        def _():
            for cp in set_copies(k0 + 1, shift=it * ns, sem=k0 + 1 + it):
                cp.wait()

        @pl.when(it == LOOP_CNT - 2)
        def _():
            for cp in set_copies(k0 + LOOP_CNT - 1):
                cp.wait()

        return carry

    jax.lax.fori_loop(0, LOOP_CNT, body, carry)
    pltpu.make_async_copy(o_buf, o_hbm, osem).wait()


@jax.jit
def pallas_standalone__layernorm_linear__sampling_kernel(
    x: jax.Array,
    g: jax.Array,
    b: jax.Array,
    w: jax.Array,
):
    B, S, D = x.shape
    xt = jnp.transpose(x, (1, 2, 0))
    no_checks = {name: True for name in ("disable_bounds_checks", "disable_semaphore_checks")
                 if hasattr(pltpu.CompilerParams, name)}
    out_t = pl.pallas_call(
        _kernel,
        in_specs=[pl.BlockSpec(memory_space=pl.ANY)] * 4,
        out_specs=pl.BlockSpec(memory_space=pl.ANY),
        out_shape=jax.ShapeDtypeStruct((2 * S, NH, B), x.dtype),
        scratch_shapes=[
            pltpu.VMEM((S, D, B), BF16),
            pltpu.VMEM((2 * S, NH, B), BF16),
            pltpu.VMEM((D, D), BF16),
            pltpu.VMEM((D,), BF16),
            pltpu.VMEM((D,), BF16),
            pltpu.VMEM((49, NQ // 2, T), U32),
            pltpu.VMEM((NH, T), U32),
            pltpu.VMEM((14, NH, T), F32),
            pltpu.VMEM((LOOP_N, 16, T, T), F32),
            pltpu.SemaphoreType.DMA((len(RAMP) + LOOP_CNT + 4,)),
            pltpu.SemaphoreType.DMA(()),
        ],
        compiler_params=pltpu.CompilerParams(vmem_limit_bytes=110 * 1024 * 1024, **no_checks),
    )(xt, g, b, w)
    return jnp.transpose(out_t.reshape(S, D, B), (2, 0, 1))
```

```python
import jax
import jax.numpy as jnp
import jax.experimental.pallas as pl
import jax.experimental.pallas.tpu as pltpu

EPS = 1e-5
F32 = jnp.float32
BF16 = jnp.bfloat16
U32 = jnp.uint32

T = 128
H = 256
NH = 288
NQ = 144
KR = 80
SGW = 512

B_TERMS = {1: ((1, 0, 0), (1, 1, 1)), 2: ((1, 0, 0),), 3: ((1, 0, 1), (1, 1, 1)), 4: ((1, 1, 0), (1, 0, 0)),
           5: ((1, 1, 1),), 6: ((1, 0, 0), (-1, 0, 1)), 7: ((1, 1, 0), (-1, 1, 1))}
A_TERMS = {1: ((1, 0, 0), (-1, 1, 1)), 2: ((1, 1, 0), (-1, 1, 1)), 3: ((1, 0, 0),), 4: ((1, 1, 1),),
           5: ((1, 0, 0), (-1, 0, 1)), 6: ((1, 1, 0), (-1, 0, 0)), 7: ((1, 0, 1), (-1, 1, 1))}
C_TERMS = {(0, 0): {1: 1, 4: 1, 5: -1, 7: 1}, (0, 1): {3: 1, 5: -1},
           (1, 0): {2: 1, 4: 1}, (1, 1): {1: -1, 2: 1, 3: 1, 6: -1}}

OUTER = (5, 2, 3, 4, 1, 6, 7)
INNER = ((2, 1, 6, 3), (5, 7, 4))
SWAP = (3, 4, 6, 7)
N_EARLY = 2

RAMP = (1, 1, 2, 4)
LOOP_N, LOOP_CNT = 8, 7
W_ITER, W_POS = 2, 2
W_ROWS = 32


def _dot(a, b):
    return jnp.dot(a, b, preferred_element_type=F32)


def _lin(terms):
    terms = sorted(terms, key=lambda t: -t[0])
    assert terms[0][0] > 0
    acc = terms[0][1]
    for sg, v in terms[1:]:
        acc = acc + v if sg > 0 else acc - v
    return acc


def _make_plan(d, last):
    rounds = [[(i, u) for u in us] for i in OUTER for us in INNER]
    if last:
        rounds = rounds[:-2] + [[("R", 1, 0)], [("R", 1, 1)]] + rounds[-2:] + [[("R", 0, 0)], [("R", 0, 1)]]
    else:
        rounds += [[("R", nh, gq)] for gq in range(2) for nh in range(2)]
    slots = []
    for rnd in rounds:
        for nm in rnd:
            if nm[0] == "R":
                key, wt = ("R", nm[2]), 3.0
            else:
                pos = OUTER.index(nm[0])
                key, wt = nm, (1.2 if pos >= 4 else float(pos > 0 and nm[1] in INNER[1]))
            if all(key != k for k, _ in slots):
                slots += [(key, wt)] * 2
    steps = d // 8
    scale = 2 * steps / sum(wt for _, wt in slots)
    pieces, acc, done = {}, 0.0, 0
    for key, wt in slots:
        acc += wt * scale
        take = int(round(acc)) - done
        if done < steps:
            take = min(take, steps - done)
        pieces.setdefault(key, []).append((min(done // steps, 1), 8 * take))
        done += take
    assert done == 2 * steps
    return rounds, pieces


def _kernel(x_hbm, g_hbm, b_hbm, w_hbm, o_hbm,
            x_buf, o_buf, w_buf, g_buf, b_buf, a_sc, ar_sc, m_sc, xn_sc, isem, osem):
    S, D, B = x_hbm.shape
    sps = B // SGW
    nsg = S * sps
    plans = {last: _make_plan(D, last) for last in (False, True)}

    blocks, g = [], 0
    for n in RAMP + (LOOP_N,) * LOOP_CNT:
        blocks.append((g, n))
        g += n
    assert g == nsg and sum(RAMP) % sps == 0 and LOOP_N == 4 * sps == 8
    sets, have = [], 0
    for bi, (g0, n) in enumerate(blocks):
        need = min(g0 + n + (bi > 0), nsg)
        sets.append((have, need))
        have = need

    def x_copy(idx, sem):
        return pltpu.make_async_copy(x_hbm.at[idx], x_buf.at[idx], isem.at[sem])

    def set_copies(k, shift=0, sem=None):
        out, g = [], sets[k][0]
        while g < sets[k][1]:
            s, j = divmod(g, sps)
            if j == 0 and sets[k][1] - g >= sps:
                ns = (sets[k][1] - g) // sps if k >= len(RAMP) else 1
                out.append(x_copy((pl.ds(s + shift, ns),), k if sem is None else sem))
                g += ns * sps
            else:
                out.append(x_copy((s + shift, slice(None), pl.ds(j * SGW, SGW)), k if sem is None else sem))
                g += 1
        return out

    def first_copies():
        return [x_copy((0, slice(None), pl.ds(gq * 2 * T, 2 * T)), (len(sets), 0)[gq]) for gq in range(2)]

    param_copies = [pltpu.make_async_copy(src, dst, isem.at[len(sets) + 1 + i])
                    for i, (src, dst) in enumerate(((w_hbm, w_buf), (g_hbm, g_buf), (b_hbm, b_buf)))]
    for cp in param_copies + first_copies():
        cp.start()
    for k in range(1, len(sets)):
        for cp in set_copies(k):
            cp.start()
    for cp in param_copies:
        cp.wait()

    w = w_buf[...]
    row16 = jax.lax.broadcasted_iota(jnp.int32, (16, D), 0)
    b16 = jnp.where(row16 == 0, b_buf[...].astype(F32).reshape(1, D), 0.0).astype(BF16)
    d_row = _dot(b16, w)[0:1, :]
    d_hi = d_row.astype(BF16).astype(F32)
    d_lo = (d_row - d_hi).astype(BF16).astype(F32)
    n_ext = 2 * H + T - D
    row_e = jax.lax.broadcasted_iota(jnp.int32, (n_ext, D), 0)
    ext = jnp.where(row_e == 0, d_hi, jnp.where(row_e == 1, d_lo, 0.0))
    wt = jnp.concatenate([w.astype(F32), ext], axis=0).T
    gf = g_buf[...].astype(F32).reshape(1, D)
    a = wt[:, :2 * H] * gf[:, :2 * H]
    a_idx = lambda i, u: OUTER.index(i) * 7 + u - 1

    def prep_left(i):
        ai = _lin([(sg, a[nh * NH:(nh + 1) * NH, kh * H:(kh + 1) * H]) for sg, nh, kh in A_TERMS[i]])
        for u in range(1, 8):
            au = _lin([(sg, ai[nh * NQ:(nh + 1) * NQ, kh * T:(kh + 1) * T]) for sg, nh, kh in A_TERMS[u]])
            a_sc[a_idx(i, u)] = pltpu.bitcast(au.astype(BF16), U32)

    for i in OUTER[:N_EARLY]:
        prep_left(i)
    g_rem = jnp.concatenate([gf[:, 2 * H:], jnp.ones((1, n_ext), F32)], axis=1)
    ar_sc[...] = pltpu.bitcast((wt[:, 2 * H:] * g_rem).astype(BF16), U32)

    class Stats:
        def __init__(self, s, c0):
            self.s, self.cs, self.r = s, slice(c0, c0 + 2 * T), 0

        def piece(self, nrows):
            for r in range(self.r, self.r + nrows, 8):
                x = x_buf[self.s, r:r + 8, self.cs].astype(F32)
                if r == 0:
                    self.c = x[0:1, :]
                y = x - self.c
                self.a1 = y if r == 0 else self.a1 + y
                self.a2 = y * y if r == 0 else self.a2 + y * y
            self.r += nrows
            z = self.a1 + self.a2
            return z[:, :T] + z[:, T:]

        def final(self):
            assert self.r == D
            s1 = jnp.sum(self.a1, axis=0, keepdims=True) * (1.0 / D)
            s2 = jnp.sum(self.a2, axis=0, keepdims=True) * (1.0 / D)
            rs = jax.lax.rsqrt(jnp.maximum(s2 - s1 * s1, 0.0) + EPS)
            return rs, (self.c + s1) * rs

        def whole(self):
            self.piece(D)
            return self.final()

    def super_group(s, c0, slot, st4, nxt, after_half):
        rounds, pieces = plans[after_half is not None]
        half = lambda v, t: v[:, (t % 2) * T:(t % 2 + 1) * T]
        r = [jnp.broadcast_to(half(st4[2 * (t // 2)], t), (8, T)) for t in range(4)]
        q = [half(st4[2 * (t // 2) + 1], t) for t in range(4)]
        always = r[0] > 0

        def normalised(r0, nr, t):
            cc = c0 + (t // 2) * 2 * T
            x = half(x_buf[s, r0:r0 + nr, cc:cc + 2 * T].astype(F32), t)
            return (x.reshape(nr // 8, 8, T) * r[t][None]).reshape(nr, T) - q[t]

        in_round, in_mem = {}, set()

        def xhat(kb, t):
            if (kb, t) not in in_round:
                if (kb, t) in in_mem:
                    in_round[(kb, t)] = xn_sc[slot, kb * 4 + t]
                else:
                    in_round[(kb, t)] = normalised(kb * T, T, t)
                    xn_sc[slot, kb * 4 + t] = in_round[(kb, t)]
                    in_mem.add((kb, t))
            return in_round[(kb, t)]

        def rounded(val, key):
            if nxt is not None:
                cr = val.shape[0] // 2
                segs = []
                for k in (1, 0):
                    si, n = pieces[key][1 - k]
                    lo = (k + 1) * cr - 8
                    tied = jnp.where(always, val[lo:lo + 8], nxt[si].piece(n)) if n else val[lo:lo + 8]
                    segs = [val[k * cr:lo], tied] + segs
                if any(n for _, n in pieces[key]):
                    val = jnp.concatenate(segs, axis=0)
            return val.astype(BF16)

        rem_operand = {}
        m_idx = lambda i, gq: OUTER.index(i) * 2 + gq
        for rnd in rounds:
            in_round.clear()
            if rnd[0][0] == "R":
                _, nh, gq = rnd[0]
                if gq not in rem_operand:
                    bt = [normalised(2 * H, D - 2 * H, 2 * gq + ch) for ch in range(2)]
                    bt = jnp.concatenate([rounded(bt[0], ("R", gq)), bt[1].astype(BF16)], axis=1)
                    ones = jnp.ones((KR - (D - 2 * H), 2 * T), BF16)
                    rem_operand[gq] = jnp.concatenate([bt, ones], axis=0)
                ar = pltpu.bitcast(ar_sc[nh * NH // 2:(nh + 1) * NH // 2, 0:KR], BF16)
                res = _dot(ar, rem_operand[gq])
                pair = [_lin([(1, half(res, ch))] + [(C_TERMS[(nh, ch)][i], m_sc[m_idx(i, gq)])
                                                     for i in OUTER if i in C_TERMS[(nh, ch)]])
                        for ch in range(2)]
                cc = c0 + gq * 2 * T
                o_buf[2 * s + nh, :, cc:cc + 2 * T] = jnp.concatenate(pair, axis=1).astype(BF16)
                if after_half is not None and gq == 1:
                    after_half(nh)
                continue
            i = rnd[0][0]
            sw = int(i in SWAP)
            res = {}
            for _, u in rnd:
                val = _lin([(s2, _lin([(s1, xhat(2 * kh + k2, 2 * (g2 ^ sw) + ch)) for s1, kh, ch in B_TERMS[i]]))
                            for s2, k2, g2 in B_TERMS[u]])
                res[u] = _dot(pltpu.bitcast(a_sc[a_idx(i, u)], BF16), rounded(val, (i, u)))
            for nh in range(2):
                for gq in range(2):
                    ct = C_TERMS[(nh, gq ^ sw)]
                    terms = [(ct[u], res[u]) for _, u in rnd if u in ct]
                    if not terms:
                        continue
                    if rnd[0][1] != INNER[0][0]:
                        terms.append((2, m_sc[m_idx(i, gq), nh * NQ:(nh + 1) * NQ, :]))
                    m_sc[m_idx(i, gq), nh * NQ:(nh + 1) * NQ, :] = _lin(terms)

    def out_copy(*idx):
        return pltpu.make_async_copy(o_buf.at[idx], o_hbm.at[idx], osem)

    def write_slabs(cond, s0, n):
        for r in range(0, NH, W_ROWS):
            pl.when(cond)(out_copy(pl.ds(2 * s0, 2 * n), pl.ds(r, W_ROWS)).start)

    def block(s_base, j_base, n, carry, look_ahead=True, it=None):
        for u in range(n):
            ds, j = divmod(j_base + u, sps)
            ds2, j2 = divmod(j_base + u + 1, sps)
            s, s2 = s_base + ds, s_base + ds2
            if u + 1 == n and it is not None:
                s2 = jnp.minimum(s2, S - 1)
            nxt = None
            if look_ahead or u + 1 < n:
                nxt = [Stats(s2, j2 * SGW), Stats(s2, j2 * SGW + 2 * T)]
            after_half = None
            if it is not None:
                final = it == LOOP_CNT - 1
                steady = jnp.logical_and(it >= W_ITER, it < LOOP_CNT - 1)
                if 0 <= u - W_POS < W_ITER + 1:
                    write_slabs(it == W_ITER, 4 * (u - W_POS), 4)
                if u == n - 1:
                    def after_half(nh):
                        for gq in range(2):
                            cols = pl.ds(j * SGW + gq * 2 * T, 2 * T)
                            pl.when(final)(out_copy(2 * s + nh, slice(None), cols).start)
            super_group(s, j * SGW, u, carry, nxt, after_half)
            if nxt is not None:
                carry = nxt[0].final() + nxt[1].final()
            if it is not None:
                if u in (1, 3, 5):
                    write_slabs(final, s, 1)
                if u in (3, 7):
                    write_slabs(steady, s - 1, 2)
                if u == 6:
                    for gq in range(2):
                        pl.when(final)(out_copy(pl.ds(2 * s, 2), slice(None), pl.ds(gq * 2 * T, 2 * T)).start)
        return carry

    assert sum(RAMP) == LOOP_N and W_POS <= 3 and W_POS + W_ITER < LOOP_N
    carry = ()
    for gq, cp in enumerate(first_copies()):
        cp.wait()
        carry += Stats(0, gq * 2 * T).whole()
    for i in OUTER[N_EARLY:]:
        prep_left(i)
    for bi in range(len(RAMP)):
        g0, n = blocks[bi]
        if bi == 1:
            carry = sum((Stats(g0 // sps, (g0 % sps) * SGW + gq * 2 * T).whole() for gq in range(2)), ())
        carry = block(g0 // sps, g0 % sps, n, carry, look_ahead=bi > 0)
        for cp in set_copies(bi + 1):
            cp.wait()
    k0, ns = len(RAMP), LOOP_N // sps

    def body(it, carry):
        carry = block(sum(RAMP) // sps + it * ns, 0, LOOP_N, carry, it=it)

        @pl.when(it < LOOP_CNT - 2)
        def _():
            for cp in set_copies(k0 + 1, shift=it * ns, sem=k0 + 1 + it):
                cp.wait()

        @pl.when(it == LOOP_CNT - 2)
        def _():
            for cp in set_copies(k0 + LOOP_CNT - 1):
                cp.wait()

        return carry

    jax.lax.fori_loop(0, LOOP_CNT, body, carry)
    pltpu.make_async_copy(o_buf, o_hbm, osem).wait()


@jax.jit
def pallas_standalone__layernorm_linear__sampling_kernel(
    x: jax.Array,
    g: jax.Array,
    b: jax.Array,
    w: jax.Array,
):
    B, S, D = x.shape
    xt = jnp.transpose(x, (1, 2, 0))
    no_checks = {name: True for name in ("disable_bounds_checks", "disable_semaphore_checks")
                 if hasattr(pltpu.CompilerParams, name)}
    out_t = pl.pallas_call(
        _kernel,
        in_specs=[pl.BlockSpec(memory_space=pl.ANY)] * 4,
        out_specs=pl.BlockSpec(memory_space=pl.ANY),
        out_shape=jax.ShapeDtypeStruct((2 * S, NH, B), x.dtype),
        scratch_shapes=[
            pltpu.VMEM((S, D, B), BF16),
            pltpu.VMEM((2 * S, NH, B), BF16),
            pltpu.VMEM((D, D), BF16),
            pltpu.VMEM((D,), BF16),
            pltpu.VMEM((D,), BF16),
            pltpu.VMEM((49, NQ // 2, T), U32),
            pltpu.VMEM((NH, T), U32),
            pltpu.VMEM((14, NH, T), F32),
            pltpu.VMEM((LOOP_N, 16, T, T), F32),
            pltpu.SemaphoreType.DMA((len(RAMP) + LOOP_CNT + 4,)),
            pltpu.SemaphoreType.DMA(()),
        ],
        compiler_params=pltpu.CompilerParams(vmem_limit_bytes=110 * 1024 * 1024, **no_checks),
    )(xt, g, b, w)
    return jnp.transpose(out_t.reshape(S, D, B), (2, 0, 1))
```

```python
import jax
import jax.numpy as jnp
import jax.experimental.pallas as pl
import jax.experimental.pallas.tpu as pltpu

EPS = 1e-5
F32 = jnp.float32
BF16 = jnp.bfloat16
U32 = jnp.uint32

T = 128
H = 256
NH = 288
NQ = 144
KR = 80
SGW = 512

B_TERMS = {1: ((1, 0, 0), (1, 1, 1)), 2: ((1, 0, 0),), 3: ((1, 0, 1), (1, 1, 1)), 4: ((1, 1, 0), (1, 0, 0)),
           5: ((1, 1, 1),), 6: ((1, 0, 0), (-1, 0, 1)), 7: ((1, 1, 0), (-1, 1, 1))}
A_TERMS = {1: ((1, 0, 0), (-1, 1, 1)), 2: ((1, 1, 0), (-1, 1, 1)), 3: ((1, 0, 0),), 4: ((1, 1, 1),),
           5: ((1, 0, 0), (-1, 0, 1)), 6: ((1, 1, 0), (-1, 0, 0)), 7: ((1, 0, 1), (-1, 1, 1))}
C_TERMS = {(0, 0): {1: 1, 4: 1, 5: -1, 7: 1}, (0, 1): {3: 1, 5: -1},
           (1, 0): {2: 1, 4: 1}, (1, 1): {1: -1, 2: 1, 3: 1, 6: -1}}

OUTER = (5, 2, 3, 4, 1, 6, 7)
INNER = ((2, 1, 6, 3), (5, 7, 4))
SWAP = (3, 4, 6, 7)
N_EARLY = 2

RAMP = (1, 1, 2)
MID_N, MID_CNT = 4, 3
LOOP_N, LOOP_CNT = 12, 4
W_POS, W_BACK = 9, 3
W_ROWS = 32


def _dot(a, b):
    return jnp.dot(a, b, preferred_element_type=F32)


def _lin(terms):
    terms = sorted(terms, key=lambda t: -t[0])
    assert terms[0][0] > 0
    acc = terms[0][1]
    for sg, v in terms[1:]:
        acc = acc + v if sg > 0 else acc - v
    return acc


def _make_plan(d, last):
    rounds = [[(i, u) for u in us] for i in OUTER for us in INNER]
    if last:
        rounds = rounds[:-2] + [[("R", 1, 0)], [("R", 1, 1)]] + rounds[-2:] + [[("R", 0, 0)], [("R", 0, 1)]]
    else:
        rounds += [[("R", nh, gq)] for gq in range(2) for nh in range(2)]
    slots = []
    for rnd in rounds:
        for nm in rnd:
            if nm[0] == "R":
                key, wt = ("R", nm[2]), 3.0
            else:
                pos = OUTER.index(nm[0])
                key, wt = nm, (1.2 if pos >= 4 else float(pos > 0 and nm[1] in INNER[1]))
            if all(key != k for k, _ in slots):
                slots += [(key, wt)] * 2
    steps = d // 8
    scale = 2 * steps / sum(wt for _, wt in slots)
    pieces, acc, done = {}, 0.0, 0
    for key, wt in slots:
        acc += wt * scale
        take = int(round(acc)) - done
        if done < steps:
            take = min(take, steps - done)
        pieces.setdefault(key, []).append((min(done // steps, 1), 8 * take))
        done += take
    assert done == 2 * steps
    return rounds, pieces


def _kernel(x_hbm, g_hbm, b_hbm, w_hbm, o_hbm,
            x_buf, o_buf, w_buf, g_buf, b_buf, a_sc, ar_sc, m_sc, xn_sc, isem, osem):
    S, D, B = x_hbm.shape
    sps = B // SGW
    nsg = S * sps
    plans = {last: _make_plan(D, last) for last in (False, True)}

    blocks, g = [], 0
    for n in RAMP + (MID_N,) * MID_CNT + (LOOP_N,) * LOOP_CNT:
        blocks.append((g, n))
        g += n
    assert g == nsg and sum(RAMP) % sps == 0 and MID_N % sps == 0 and LOOP_N % (2 * sps) == 0
    sets, have = [], 0
    for bi, (g0, n) in enumerate(blocks):
        need = min(g0 + n + (bi > 0), nsg)
        sets.append((have, need))
        have = need

    def x_copy(idx, sem):
        return pltpu.make_async_copy(x_hbm.at[idx], x_buf.at[idx], isem.at[sem])

    def set_copies(k, shift=0, sem=None):
        out, g = [], sets[k][0]
        while g < sets[k][1]:
            s, j = divmod(g, sps)
            if j == 0 and sets[k][1] - g >= sps:
                ns = (sets[k][1] - g) // sps if k >= len(RAMP) else 1
                out.append(x_copy((pl.ds(s + shift, ns),), k if sem is None else sem))
                g += ns * sps
            else:
                out.append(x_copy((s + shift, slice(None), pl.ds(j * SGW, SGW)), k if sem is None else sem))
                g += 1
        return out

    def first_copies():
        return [x_copy((0, slice(None), pl.ds(gq * 2 * T, 2 * T)), (len(sets), 0)[gq]) for gq in range(2)]

    param_copies = [pltpu.make_async_copy(src, dst, isem.at[len(sets) + 1 + i])
                    for i, (src, dst) in enumerate(((w_hbm, w_buf), (g_hbm, g_buf), (b_hbm, b_buf)))]
    for cp in param_copies + first_copies():
        cp.start()
    for k in range(1, len(sets)):
        for cp in set_copies(k):
            cp.start()
    for cp in param_copies:
        cp.wait()

    w = w_buf[...]
    row16 = jax.lax.broadcasted_iota(jnp.int32, (16, D), 0)
    b16 = jnp.where(row16 == 0, b_buf[...].astype(F32).reshape(1, D), 0.0).astype(BF16)
    d_row = _dot(b16, w)[0:1, :]
    d_hi = d_row.astype(BF16).astype(F32)
    d_lo = (d_row - d_hi).astype(BF16).astype(F32)
    n_ext = 2 * H + T - D
    row_e = jax.lax.broadcasted_iota(jnp.int32, (n_ext, D), 0)
    ext = jnp.where(row_e == 0, d_hi, jnp.where(row_e == 1, d_lo, 0.0))
    wt = jnp.concatenate([w.astype(F32), ext], axis=0).T
    gf = g_buf[...].astype(F32).reshape(1, D)
    a = wt[:, :2 * H] * gf[:, :2 * H]
    a_idx = lambda i, u: OUTER.index(i) * 7 + u - 1

    def prep_left(i):
        ai = _lin([(sg, a[nh * NH:(nh + 1) * NH, kh * H:(kh + 1) * H]) for sg, nh, kh in A_TERMS[i]])
        for u in range(1, 8):
            au = _lin([(sg, ai[nh * NQ:(nh + 1) * NQ, kh * T:(kh + 1) * T]) for sg, nh, kh in A_TERMS[u]])
            a_sc[a_idx(i, u)] = pltpu.bitcast(au.astype(BF16), U32)

    for i in OUTER[:N_EARLY]:
        prep_left(i)
    g_rem = jnp.concatenate([gf[:, 2 * H:], jnp.ones((1, n_ext), F32)], axis=1)
    ar_sc[...] = pltpu.bitcast((wt[:, 2 * H:] * g_rem).astype(BF16), U32)

    class Stats:
        def __init__(self, s, c0):
            self.s, self.cs, self.r = s, slice(c0, c0 + 2 * T), 0

        def piece(self, nrows):
            for r in range(self.r, self.r + nrows, 8):
                x = x_buf[self.s, r:r + 8, self.cs].astype(F32)
                if r == 0:
                    self.c = x[0:1, :]
                y = x - self.c
                self.a1 = y if r == 0 else self.a1 + y
                self.a2 = y * y if r == 0 else self.a2 + y * y
            self.r += nrows
            z = self.a1 + self.a2
            return z[:, :T] + z[:, T:]

        def final(self):
            assert self.r == D
            s1 = jnp.sum(self.a1, axis=0, keepdims=True) * (1.0 / D)
            s2 = jnp.sum(self.a2, axis=0, keepdims=True) * (1.0 / D)
            rs = jax.lax.rsqrt(jnp.maximum(s2 - s1 * s1, 0.0) + EPS)
            return rs, (self.c + s1) * rs

        def whole(self):
            self.piece(D)
            return self.final()

    def super_group(s, c0, slot, st4, nxt, after_half):
        rounds, pieces = plans[after_half is not None]
        half = lambda v, t: v[:, (t % 2) * T:(t % 2 + 1) * T]
        r = [jnp.broadcast_to(half(st4[2 * (t // 2)], t), (8, T)) for t in range(4)]
        q = [half(st4[2 * (t // 2) + 1], t) for t in range(4)]
        always = r[0] >= 0

        def normalised(r0, nr, t):
            cc = c0 + (t // 2) * 2 * T
            x = half(x_buf[s, r0:r0 + nr, cc:cc + 2 * T].astype(F32), t)
            return (x.reshape(nr // 8, 8, T) * r[t][None]).reshape(nr, T) - q[t]

        in_round, in_mem = {}, set()

        def xhat(kb, t):
            if (kb, t) not in in_round:
                if (kb, t) in in_mem:
                    in_round[(kb, t)] = xn_sc[slot, kb * 4 + t]
                else:
                    in_round[(kb, t)] = normalised(kb * T, T, t)
                    xn_sc[slot, kb * 4 + t] = in_round[(kb, t)]
                    in_mem.add((kb, t))
            return in_round[(kb, t)]

        def rounded(val, key):
            if nxt is not None:
                cr = val.shape[0] // 2
                segs = []
                for k in (1, 0):
                    si, n = pieces[key][1 - k]
                    lo = (k + 1) * cr - 8
                    tied = jnp.where(always, val[lo:lo + 8], nxt[si].piece(n)) if n else val[lo:lo + 8]
                    segs = [val[k * cr:lo], tied] + segs
                if any(n for _, n in pieces[key]):
                    val = jnp.concatenate(segs, axis=0)
            return val.astype(BF16)

        rem_operand = {}
        m_idx = lambda i, gq: OUTER.index(i) * 2 + gq
        for rnd in rounds:
            in_round.clear()
            if rnd[0][0] == "R":
                _, nh, gq = rnd[0]
                if gq not in rem_operand:
                    bt = [normalised(2 * H, D - 2 * H, 2 * gq + ch) for ch in range(2)]
                    bt = jnp.concatenate([rounded(bt[0], ("R", gq)), bt[1].astype(BF16)], axis=1)
                    ones = jnp.ones((KR - (D - 2 * H), 2 * T), BF16)
                    rem_operand[gq] = jnp.concatenate([bt, ones], axis=0)
                ar = pltpu.bitcast(ar_sc[nh * NH // 2:(nh + 1) * NH // 2, 0:KR], BF16)
                res = _dot(ar, rem_operand[gq])
                pair = [_lin([(1, half(res, ch))] + [(C_TERMS[(nh, ch)][i], m_sc[m_idx(i, gq)])
                                                     for i in OUTER if i in C_TERMS[(nh, ch)]])
                        for ch in range(2)]
                cc = c0 + gq * 2 * T
                o_buf[2 * s + nh, :, cc:cc + 2 * T] = jnp.concatenate(pair, axis=1).astype(BF16)
                if after_half is not None and gq == 1:
                    after_half(nh)
                continue
            i = rnd[0][0]
            sw = int(i in SWAP)
            res = {}
            for _, u in rnd:
                val = _lin([(s2, _lin([(s1, xhat(2 * kh + k2, 2 * (g2 ^ sw) + ch)) for s1, kh, ch in B_TERMS[i]]))
                            for s2, k2, g2 in B_TERMS[u]])
                res[u] = _dot(pltpu.bitcast(a_sc[a_idx(i, u)], BF16), rounded(val, (i, u)))
            for nh in range(2):
                for gq in range(2):
                    ct = C_TERMS[(nh, gq ^ sw)]
                    terms = [(ct[u], res[u]) for _, u in rnd if u in ct]
                    if not terms:
                        continue
                    if rnd[0][1] != INNER[0][0]:
                        terms.append((2, m_sc[m_idx(i, gq), nh * NQ:(nh + 1) * NQ, :]))
                    m_sc[m_idx(i, gq), nh * NQ:(nh + 1) * NQ, :] = _lin(terms)

    def out_copy(*idx):
        return pltpu.make_async_copy(o_buf.at[idx], o_hbm.at[idx], osem)

    def write_slabs(cond, s0, n):
        for r in range(0, NH, W_ROWS):
            pl.when(cond)(out_copy(pl.ds(2 * s0, 2 * n), pl.ds(r, W_ROWS)).start)

    pre = (sum(RAMP) + MID_N * MID_CNT) // sps
    n_back = 4 * W_BACK - pre
    assert n_back % 2 == 0 and n_back * sps <= W_POS + W_BACK - 1 < LOOP_N

    def block(s_base, j_base, n, carry, look_ahead=True, it=None):
        for u in range(n):
            ds, j = divmod(j_base + u, sps)
            ds2, j2 = divmod(j_base + u + 1, sps)
            s, s2 = s_base + ds, s_base + ds2
            if u + 1 == n and it is not None:
                s2 = jnp.minimum(s2, S - 1)
            nxt = None
            if look_ahead or u + 1 < n:
                nxt = [Stats(s2, j2 * SGW), Stats(s2, j2 * SGW + 2 * T)]
            after_half = None
            if it is not None:
                final = it == LOOP_CNT - 1
                if 0 <= u - W_POS < W_BACK:
                    write_slabs(it == 0, 4 * (u - W_POS), 4)
                if u == n - 1:
                    def after_half(nh):
                        for gq in range(2):
                            cols = pl.ds(j * SGW + gq * 2 * T, 2 * T)
                            pl.when(final)(out_copy(2 * s + nh, slice(None), cols).start)
            super_group(s, j * SGW, u, carry, nxt, after_half)
            if nxt is not None:
                carry = nxt[0].final() + nxt[1].final()
            if it is not None:
                tail = ds >= n // sps - 4
                if j == sps - 1 and tail and u < n - 1:
                    write_slabs(final, s, 1)
                if j == sps - 1 and ds % 2 == 1:
                    write_slabs(jnp.logical_and(it >= int(ds < n_back), it < LOOP_CNT - int(tail)), s - 1, 2)
                if u == n - 2:
                    for gq in range(2):
                        pl.when(final)(out_copy(pl.ds(2 * s, 2), slice(None), pl.ds(gq * 2 * T, 2 * T)).start)
        return carry

    carry = ()
    for gq, cp in enumerate(first_copies()):
        cp.wait()
        carry += Stats(0, gq * 2 * T).whole()
    for i in OUTER[N_EARLY:]:
        prep_left(i)
    for bi in range(len(RAMP)):
        g0, n = blocks[bi]
        if bi == 1:
            carry = sum((Stats(g0 // sps, (g0 % sps) * SGW + gq * 2 * T).whole() for gq in range(2)), ())
        carry = block(g0 // sps, g0 % sps, n, carry, look_ahead=bi > 0)
        for cp in set_copies(bi + 1):
            cp.wait()

    def wait_shifted(cond, k, it, n):
        @pl.when(cond)
        def _():
            for cp in set_copies(k, shift=it * (n // sps), sem=k + it):
                cp.wait()

    k1, k2 = len(RAMP), len(RAMP) + MID_CNT

    def mid_body(it, carry):
        carry = block(sum(RAMP) // sps + it * (MID_N // sps), 0, MID_N, carry)
        wait_shifted(it < MID_CNT - 1, k1 + 1, it, MID_N)
        return carry

    carry = jax.lax.fori_loop(0, MID_CNT, mid_body, carry)
    for cp in set_copies(k2):
        cp.wait()

    def body(it, carry):
        carry = block(pre + it * (LOOP_N // sps), 0, LOOP_N, carry, it=it)
        wait_shifted(it < LOOP_CNT - 2, k2 + 1, it, LOOP_N)
        wait_shifted(it == LOOP_CNT - 2, k2 + LOOP_CNT - 1, 0, LOOP_N)
        return carry

    jax.lax.fori_loop(0, LOOP_CNT, body, carry)
    pltpu.make_async_copy(o_buf, o_hbm, osem).wait()


@jax.jit
def pallas_standalone__layernorm_linear__sampling_kernel(
    x: jax.Array,
    g: jax.Array,
    b: jax.Array,
    w: jax.Array,
):
    B, S, D = x.shape
    xt = jnp.transpose(x, (1, 2, 0))
    no_checks = {name: True for name in ("disable_bounds_checks", "disable_semaphore_checks")
                 if hasattr(pltpu.CompilerParams, name)}
    out_t = pl.pallas_call(
        _kernel,
        in_specs=[pl.BlockSpec(memory_space=pl.ANY)] * 4,
        out_specs=pl.BlockSpec(memory_space=pl.ANY),
        out_shape=jax.ShapeDtypeStruct((2 * S, NH, B), x.dtype),
        scratch_shapes=[
            pltpu.VMEM((S, D, B), BF16),
            pltpu.VMEM((2 * S, NH, B), BF16),
            pltpu.VMEM((D, D), BF16),
            pltpu.VMEM((D,), BF16),
            pltpu.VMEM((D,), BF16),
            pltpu.VMEM((49, NQ // 2, T), U32),
            pltpu.VMEM((NH, T), U32),
            pltpu.VMEM((14, NH, T), F32),
            pltpu.VMEM((LOOP_N, 16, T, T), F32),
            pltpu.SemaphoreType.DMA((len(RAMP) + MID_CNT + LOOP_CNT + 4,)),
            pltpu.SemaphoreType.DMA(()),
        ],
        compiler_params=pltpu.CompilerParams(vmem_limit_bytes=110 * 1024 * 1024, **no_checks),
    )(xt, g, b, w)
    return jnp.transpose(out_t.reshape(S, D, B), (2, 0, 1))
```
